```python
import jax
import jax.numpy as jnp

def _softmax(x, axis=-1):
    return jax.nn.softmax(x, axis=axis)

def _gelu(x):
    return jax.nn.gelu(x, approximate=True)

def _silu(x):
    return jax.nn.silu(x)

def _sigmoid(x):
    return jax.nn.sigmoid(x)

def _layernorm(x, axis=-1, eps=1e-05):
    m = jnp.mean(x, axis=axis, keepdims=True)
    v = jnp.var(x, axis=axis, keepdims=True)
    return (x - m) / jnp.sqrt(v + eps)

def _scatter_add(tgt, idx, src, axis=0):
    return tgt.at[idx].add(src)

def _segment_sum(src, seg, n):
    return jax.ops.segment_sum(src, seg, n)

class _Rng:

    def __init__(self, key):
        self._k = key

    def _next(self):
        self._k, sub = jax.random.split(self._k)
        return sub

    def normal(self, shape):
        return jax.random.normal(self._next(), shape, dtype=jnp.bfloat16)

    def randint(self, lo, hi, shape):
        return jax.random.randint(self._next(), shape, lo, hi, dtype=jnp.int32)

    def uniform(self, shape, lo=0.0, hi=1.0):
        return jax.random.uniform(self._next(), shape, jnp.bfloat16, lo, hi)

    def permutation(self, n):
        return jax.random.permutation(self._next(), n)
kernel_name = 'gated_mix__memory_aug_recurrent_mem_tr__sliding_local_dilated__prompt'

def setup_inputs():
    _rng = _Rng(jax.random.key(int.from_bytes(__import__("os").urandom(4), "little")))
    _w = lambda a: (lambda t: t.astype(jnp.bfloat16) if jnp.issubdtype(t.dtype, jnp.floating) else t)(jnp.asarray(a))

    def _A_setup():
        B, S, Dm = (1, 2048, 640)
        H, Dh = (32, 192)
        M, seg = (8, 32)
        seg = min(seg, S)
        S = S // seg * seg
        return {'x': _w((lambda *s: _rng.normal(s) * 0.05)(B, S, Dm)), 'mem0': _w((lambda *s: _rng.normal(s) * 0.05)(B, M, Dm)), 'Wq': _w((lambda *s: _rng.normal(s) * 0.05)(Dm, H, Dh) * Dm ** (-0.5)), 'Wk': _w((lambda *s: _rng.normal(s) * 0.05)(Dm, H, Dh) * Dm ** (-0.5)), 'Wv': _w((lambda *s: _rng.normal(s) * 0.05)(Dm, H, Dh) * Dm ** (-0.5)), 'Wo': _w((lambda *s: _rng.normal(s) * 0.05)(H, Dh, Dm) * (H * Dh) ** (-0.5)), 'seg_len': seg}
    _A_in = _A_setup()

    def _B_setup():
        B, S, D = (1, 2048, 640)
        return {'x': _w((lambda *s: _rng.normal(s) * 0.05)(B, S, D)), 'wqkv': _w((lambda *s: _rng.normal(s) * 0.05)(D, 3 * D)), 'wo': _w((lambda *s: _rng.normal(s) * 0.05)(D, D))}
    _B_in = _B_setup()
    return {'A_x': _A_in['x'], 'A_mem0': _A_in['mem0'], 'A_Wq': _A_in['Wq'], 'A_Wk': _A_in['Wk'], 'A_Wv': _A_in['Wv'], 'A_Wo': _A_in['Wo'], 'A_seg_len': _A_in['seg_len'], 'B_x': _B_in['x'], 'B_wqkv': _B_in['wqkv'], 'B_wo': _B_in['wo'], 'gate_w': _w((lambda *s: _rng.normal(s) * 0.05)(640))}

def reference(A_x, A_mem0, A_Wq, A_Wk, A_Wv, A_Wo, A_seg_len, B_x, B_wqkv, B_wo, gate_w):

    def _A_ref(x, mem0, Wq, Wk, Wv, Wo, seg_len):
        B, S, Dm = x.shape
        H, Dh = (Wq.shape[1], Wq.shape[2])
        M = mem0.shape[1]
        scale = Dh ** (-0.5)
        n_seg = S // seg_len
        L = M + seg_len
        idx = jnp.arange(L)
        mask = (idx[:, None] < M) | (idx[:, None] >= idx[None, :])
        mem = mem0
        outs = []
        for s in range(n_seg):
            xs = x[:, s * seg_len:(s + 1) * seg_len, :].copy()
            h = jnp.concatenate([mem, xs], axis=1)
            q = jnp.einsum('btd,dhe->bhte', h, Wq)
            k = jnp.einsum('btd,dhe->bhte', h, Wk)
            v = jnp.einsum('btd,dhe->bhte', h, Wv)
            scores = jnp.einsum('bhqe,bhke->bhqk', q, k) * scale
            scores = jnp.where(mask[None, None], scores, -1000000000.0)
            p = _softmax(scores, axis=-1)
            o = jnp.einsum('bhqk,bhke->bhqe', p, v)
            o = jnp.einsum('bhte,hed->btd', o, Wo)
            mem = o[:, :M, :].copy()
            outs.append(o[:, M:, :])
        return jnp.concatenate(outs, axis=1)

    def _B_ref(x, wqkv, wo):
        B, S, D = x.shape
        H = 32
        Dh = D // H
        W, dil = (8, 2)
        qkv = (lambda x, *d: x.transpose(*d))((x @ wqkv).reshape(B, S, 3, H, Dh), 2, 0, 3, 1, 4)
        q, k, v = (qkv[0], qkv[1], qkv[2])
        scale = Dh ** (-0.5)
        pos = jnp.arange(S)
        off = jnp.arange(W) * dil
        idx = pos[:, None] - off[None, :]
        mask = idx >= 0
        idx_c = jnp.where(mask, idx, 0).reshape(-1)
        kg = k[:, :, idx_c, :].reshape(B, H, S, W, Dh)
        vg = v[:, :, idx_c, :].reshape(B, H, S, W, Dh)
        logits = jnp.einsum('bhsd,bhswd->bhsw', q, kg) * scale
        logits = jnp.where(mask[None, None, :, :], logits, -1000000000.0)
        attn = _softmax(logits, axis=-1)
        o = jnp.einsum('bhsw,bhswd->bhsd', attn, vg)
        return (lambda x, *d: x.transpose(*d))(o, 0, 2, 1, 3).reshape(B, S, D) @ wo
    x = A_x
    g = _sigmoid((x * gate_w).sum(-1, keepdims=True))
    a = _A_ref(x, A_mem0, A_Wq, A_Wk, A_Wv, A_Wo, A_seg_len)
    b = _B_ref(x, B_wqkv, B_wo)
    return g * a + (1 - g) * b
```

```python
import functools

import jax
import jax.numpy as jnp
import jax.experimental.pallas as pl
import jax.experimental.pallas.tpu as pltpu

F32 = jnp.float32
BF16 = jnp.bfloat16
I32 = jnp.int32

LANES = 128
B_HEADS = 32
B_WIN = 8
B_DIL = 2
HALO = 16
NEG = -1000000000.0


def _nt(a, b):
    return jax.lax.dot_general(a, b, (((1,), (1,)), ((), ())), preferred_element_type=F32)


def _nn(a, b):
    return jax.lax.dot_general(a, b, (((1,), (0,)), ((), ())), preferred_element_type=F32)


def _pack(w):
    return pltpu.bitcast(w, I32)


def _unpack(w):
    return pltpu.bitcast(w, BF16)


def _kernel(x_hbm, mem0_ref, wq_hbm, wk_hbm, wv_hbm, wo_hbm, bqkv_hbm, bwo_hbm, gate_ref,
            out_hbm,
            x_v, bqkv_v, bwo_v, bqkv_p, bwo_p, k_scr, v_scr, g_scr, b_scr,
            stage, wqkv_p, wo_p, h_scr, o_scr, out_v,
            in_sem, w_sem, out_sem,
            *, S, D, H, Dh, M, seg, n_chunk, out_every):
    L = M + seg
    n_seg = S // seg
    n_pair = H // 2
    PW = 2 * Dh
    R = S // n_chunk
    ppc = n_pair // n_chunk
    nt = D // LANES
    dB = D // B_HEADS

    cp_bqkv = pltpu.make_async_copy(bqkv_hbm, bqkv_v, in_sem.at[0])
    cp_x = pltpu.make_async_copy(x_hbm, x_v, in_sem.at[1])
    cp_bwo = pltpu.make_async_copy(bwo_hbm, bwo_v, in_sem.at[2])
    cp_bqkv.start()
    cp_x.start()
    cp_bwo.start()

    def w_copy(c, j):
        src = (wq_hbm, wk_hbm, wv_hbm, wo_hbm)[j]
        rows = pl.ds(pl.multiple_of(c * (ppc * PW), ppc * PW), ppc * PW)
        return pltpu.make_async_copy(src.at[rows, :], stage.at[c, j], w_sem.at[c, j])

    for c in range(n_chunk):
        for j in range(4):
            w_copy(c, j).start()

    ri = jax.lax.broadcasted_iota(I32, (D, D), 0)
    ci = jax.lax.broadcasted_iota(I32, (D, D), 1)
    perm = jnp.where(ri == (ci % B_HEADS) * dB + ci // B_HEADS, 1.0, 0.0).astype(BF16)
    perm_t = jnp.where(ci == (ri % B_HEADS) * dB + ri // B_HEADS, 1.0, 0.0).astype(BF16)
    cp_bqkv.wait()
    for j in range(3):
        bqkv_p[:, j * D:(j + 1) * D] = _pack(_nn(bqkv_v[:, j * D:(j + 1) * D], perm).astype(BF16))
    cp_bwo.wait()
    bwo_p[...] = _pack(_nn(perm_t, bwo_v[...]).astype(BF16))
    cp_x.wait()

    gate = gate_ref[...].astype(F32)
    b_scale = dB ** (-0.5)

    kv0 = _nn(x_v[0:16, :], _unpack(bqkv_p[:, D:3 * D]))[0:1, :]
    for t in range(nt):
        k_scr[t, R:R + HALO, :] = jnp.broadcast_to(kv0[:, t * LANES:(t + 1) * LANES], (HALO, LANES))
        v_scr[t, R:R + HALO, :] = jnp.broadcast_to(kv0[:, D + t * LANES:D + (t + 1) * LANES], (HALO, LANES))

    def b_chunk(c, carry):
        r0 = pl.multiple_of(c * R, R)
        xb = x_v[pl.ds(r0, R), :]
        g = jax.nn.sigmoid(jnp.sum(xb.astype(F32) * gate, axis=-1, keepdims=True))
        g_scr[pl.ds(r0, R), :] = jnp.broadcast_to(g, (R, LANES))

        kk = _nn(xb, _unpack(bqkv_p[:, D:2 * D]))
        for t in range(nt):
            k_scr[t, 0:HALO, :] = k_scr[t, R:R + HALO, :]
            k_scr[t, HALO:HALO + R, :] = kk[:, t * LANES:(t + 1) * LANES]
        vv = _nn(xb, _unpack(bqkv_p[:, 2 * D:3 * D]))
        for t in range(nt):
            v_scr[t, 0:HALO, :] = v_scr[t, R:R + HALO, :]
            v_scr[t, HALO:HALO + R, :] = vv[:, t * LANES:(t + 1) * LANES]
        qq = _nn(xb, _unpack(bqkv_p[:, 0:D])) * b_scale

        pos = r0 + jax.lax.broadcasted_iota(I32, (R, LANES), 0)
        logits = []
        for w in range(B_WIN):
            off = HALO - B_DIL * w
            acc = qq[:, 0:LANES] * k_scr[0, off:off + R, :]
            for t in range(1, nt):
                acc = acc + qq[:, t * LANES:(t + 1) * LANES] * k_scr[t, off:off + R, :]
            acc = acc + pltpu.roll(acc, 64, 1)
            acc = acc + pltpu.roll(acc, 32, 1)
            if w > 0:
                acc = jnp.where(pos >= B_DIL * w, acc, NEG)
            logits.append(acc)
        mx = functools.reduce(jnp.maximum, logits)
        es = [jnp.exp(l - mx) for l in logits]
        inv = 1.0 / functools.reduce(jnp.add, es)
        outs = []
        for t in range(nt):
            acc = es[0] * v_scr[t, HALO:HALO + R, :]
            for w in range(1, B_WIN):
                off = HALO - B_DIL * w
                acc = acc + es[w] * v_scr[t, off:off + R, :]
            outs.append((acc * inv).astype(BF16))
        bb = _nn(jnp.concatenate(outs, axis=1), _unpack(bwo_p[...]))
        b_scr[pl.ds(r0, R), :] = (1.0 - g) * bb

        for j in range(4):
            w_copy(c, j).wait()
        for i in range(ppc):
            p = c * ppc + i
            for j in range(3):
                wqkv_p[p, :, j * PW:(j + 1) * PW] = _pack(stage[c, j, i * PW:(i + 1) * PW, :].T)
            wo_p[p] = _pack(stage[c, 3, i * PW:(i + 1) * PW, :])
        return carry

    jax.lax.fori_loop(0, n_chunk, b_chunk, 0)

    a_scale = Dh ** (-0.5)
    h_scr[0:M, :] = mem0_ref[...].astype(F32)

    def out_copy(i):
        rows = pl.ds(pl.multiple_of(i * (out_every * seg), out_every * seg), out_every * seg)
        return pltpu.make_async_copy(out_v.at[rows, :], out_hbm.at[rows, :], out_sem)

    def a_step(s, carry):
        r0 = pl.multiple_of(s * seg, seg)
        h_scr[M:L, :] = x_v[pl.ds(r0, seg), :].astype(F32)

        row = jax.lax.broadcasted_iota(I32, (L, 2 * L), 0)
        col = jax.lax.broadcasted_iota(I32, (L, 2 * L), 1)
        first = col < L
        key = jnp.where(first, col, col - L)
        visible = (row < M) | (row >= key)
        lane = jax.lax.broadcasted_iota(I32, (L, PW), 1)
        in_a = lane < Dh

        def block_diag(z):
            return jnp.concatenate([jnp.where(in_a, z, 0.0), jnp.where(in_a, 0.0, z)], axis=0).astype(BF16)

        def project(p):
            qkv = _nn(h_scr[...], _unpack(wqkv_p[p]))
            return qkv[:, 0:PW], block_diag(qkv[:, PW:2 * PW]), block_diag(qkv[:, 2 * PW:3 * PW])

        def attend(p, q, kbd, vbd):
            sc = jnp.where(visible, _nt(q, kbd) * a_scale, NEG)
            m_a = jnp.max(jnp.where(first, sc, -jnp.inf), axis=-1, keepdims=True)
            m_b = jnp.max(jnp.where(first, -jnp.inf, sc), axis=-1, keepdims=True)
            e = jnp.exp(sc - jnp.where(first, m_a, m_b))
            l_a = jnp.sum(jnp.where(first, e, 0.0), axis=-1, keepdims=True)
            l_b = jnp.sum(jnp.where(first, 0.0, e), axis=-1, keepdims=True)
            pr = e * jnp.where(first, 1.0 / l_a, 1.0 / l_b)
            o_scr[:, p * PW:(p + 1) * PW] = _nn(pr, vbd)

        prev = project(0)
        for p in range(1, n_pair):
            cur = project(p)
            attend(p - 1, *prev)
            prev = cur
        attend(n_pair - 1, *prev)

        acc = _nn(o_scr[:, 0:PW], _unpack(wo_p[0]))
        for p in range(1, n_pair):
            acc = acc + _nn(o_scr[:, p * PW:(p + 1) * PW], _unpack(wo_p[p]))

        h_scr[0:M, :] = acc[0:M, :]
        g = g_scr[pl.ds(r0, seg), :]
        g = jnp.concatenate([g] * nt, axis=1)
        out_v[pl.ds(r0, seg), :] = (g * acc[M:L, :] + b_scr[pl.ds(r0, seg), :]).astype(out_v.dtype)

        @pl.when(s % out_every == out_every - 1)
        def _():
            out_copy(s // out_every).start()

        return carry

    jax.lax.fori_loop(0, n_seg, a_step, 0)
    pltpu.make_async_copy(out_v, out_hbm, out_sem).wait()


@functools.partial(jax.jit, static_argnames=("A_seg_len",))
def pallas_gated_mix__memory_aug_recurrent_mem_tr__sliding_local_dilated__prompt_kernel(
    A_x: jax.Array,
    A_mem0: jax.Array,
    A_Wq: jax.Array,
    A_Wk: jax.Array,
    A_Wv: jax.Array,
    A_Wo: jax.Array,
    A_seg_len: int,
    B_x: jax.Array,
    B_wqkv: jax.Array,
    B_wo: jax.Array,
    gate_w: jax.Array,
):
    del B_x
    Bsz, S, D = A_x.shape
    _, H, Dh = A_Wq.shape
    M = A_mem0.shape[1]
    seg = int(A_seg_len)
    assert Bsz == 1 and S % seg == 0 and H % 2 == 0 and (2 * Dh) % LANES == 0 and D % LANES == 0
    n_chunk = 8
    out_every = 8
    n_pair = H // 2
    PW = 2 * Dh
    R = S // n_chunk
    L = M + seg

    def head_major(w):
        return jnp.transpose(w, (1, 2, 0)).reshape(H * Dh, D)

    any_spec = pl.BlockSpec(memory_space=pl.ANY)
    vmem_spec = pl.BlockSpec(memory_space=pltpu.VMEM)
    out = pl.pallas_call(
        functools.partial(_kernel, S=S, D=D, H=H, Dh=Dh, M=M, seg=seg,
                          n_chunk=n_chunk, out_every=out_every),
        out_shape=jax.ShapeDtypeStruct((S, D), A_x.dtype),
        in_specs=[any_spec, vmem_spec, any_spec, any_spec, any_spec, any_spec,
                  any_spec, any_spec, vmem_spec],
        out_specs=any_spec,
        scratch_shapes=[
            pltpu.VMEM((S, D), BF16),
            pltpu.VMEM((D, 3 * D), BF16),
            pltpu.VMEM((D, D), BF16),
            pltpu.VMEM((D // 2, 3 * D), I32),
            pltpu.VMEM((D // 2, D), I32),
            pltpu.VMEM((D // LANES, HALO + R, LANES), F32),
            pltpu.VMEM((D // LANES, HALO + R, LANES), F32),
            pltpu.VMEM((S, LANES), F32),
            pltpu.VMEM((S, D), F32),
            pltpu.VMEM((n_chunk, 4, n_pair // n_chunk * PW, D), BF16),
            pltpu.VMEM((n_pair, D // 2, 3 * PW), I32),
            pltpu.VMEM((n_pair, PW // 2, D), I32),
            pltpu.VMEM((L, D), F32),
            pltpu.VMEM((L, H * Dh), F32),
            pltpu.VMEM((S, D), A_x.dtype),
            pltpu.SemaphoreType.DMA((3,)),
            pltpu.SemaphoreType.DMA((n_chunk, 4)),
            pltpu.SemaphoreType.DMA(()),
        ],
        compiler_params=pltpu.CompilerParams(vmem_limit_bytes=110 * 1024 * 1024),
    )(
        A_x.reshape(S, D),
        A_mem0.reshape(M, D),
        head_major(A_Wq),
        head_major(A_Wk),
        head_major(A_Wv),
        A_Wo.reshape(H * Dh, D),
        B_wqkv,
        B_wo,
        gate_w.reshape(1, D),
    )
    return out.reshape(Bsz, S, D)
```

```python
import functools

import jax
import jax.numpy as jnp
import jax.experimental.pallas as pl
import jax.experimental.pallas.tpu as pltpu

F32 = jnp.float32
BF16 = jnp.bfloat16
I32 = jnp.int32

LANES = 128
B_HEADS = 32
B_WIN = 8
B_DIL = 2
HALO = 16
NEG = -1000000000.0
RS = 64
RA = 16
W_AHEAD = 3


def _nt(a, b):
    return jax.lax.dot_general(a, b, (((1,), (1,)), ((), ())), preferred_element_type=F32)


def _nn(a, b):
    return jax.lax.dot_general(a, b, (((1,), (0,)), ((), ())), preferred_element_type=F32)


def _pack(w):
    return pltpu.bitcast(w, I32)


def _unpack(w):
    return pltpu.bitcast(w, BF16)


def _kernel(x_hbm, mem0_ref, wq_hbm, wk_hbm, wv_hbm, wo_hbm, bqkv_hbm, bwo_hbm, gate_ref,
            out_hbm,
            x_v, bqkv_v, bwo_v, bqkv_p, bwo_p, q_scr, k_scr, v_scr, ob_scr, g_scr, b_scr,
            stage, wqkv_p, wo_p, h_scr, o_scr, out_v,
            in_sem, w_sem, out_sem,
            *, S, D, H, Dh, M, seg, n_chunk, out_every):
    L = M + seg
    n_seg = S // seg
    n_pair = H // 2
    PW = 2 * Dh
    R = S // n_chunk
    ppc = n_pair // n_chunk
    nt = D // LANES
    dB = D // B_HEADS

    def bqkv_copy(j):
        cols = pl.ds(j * D, D)
        return pltpu.make_async_copy(bqkv_hbm.at[:, cols], bqkv_v.at[j], in_sem.at[j])

    cp_x = pltpu.make_async_copy(x_hbm, x_v, in_sem.at[3])
    cp_bwo = pltpu.make_async_copy(bwo_hbm, bwo_v, in_sem.at[4])

    def w_copy(c, j):
        src = (wq_hbm, wk_hbm, wv_hbm, wo_hbm)[j]
        rows = pl.ds(pl.multiple_of(c * (ppc * PW), ppc * PW), ppc * PW)
        return pltpu.make_async_copy(src.at[rows, :], stage.at[c, j], w_sem.at[c, j])

    def w_start(c):
        for j in range(4):
            w_copy(c, j).start()

    bqkv_copy(0).start()

    ri = jax.lax.broadcasted_iota(I32, (D, D), 0)
    ci = jax.lax.broadcasted_iota(I32, (D, D), 1)
    perm = jnp.where(ri == (ci % B_HEADS) * dB + ci // B_HEADS, 1.0, 0.0).astype(BF16)
    perm_t = jnp.where(ci == (ri % B_HEADS) * dB + ri // B_HEADS, 1.0, 0.0).astype(BF16)
    bqkv_copy(0).wait()
    bqkv_copy(1).start()
    bqkv_copy(2).start()
    cp_bwo.start()
    cp_x.start()
    bqkv_p[0] = _pack(_nn(bqkv_v[0], perm).astype(BF16))
    bqkv_copy(1).wait()
    w_start(0)
    bqkv_p[1] = _pack(_nn(bqkv_v[1], perm).astype(BF16))
    bqkv_copy(2).wait()
    w_start(1)
    bqkv_p[2] = _pack(_nn(bqkv_v[2], perm).astype(BF16))
    cp_bwo.wait()
    w_start(2)
    bwo_p[...] = _pack(_nn(perm_t, bwo_v[...]).astype(BF16))
    cp_x.wait()

    gate = gate_ref[...].astype(F32)
    b_scale = dB ** (-0.5)

    k0 = _nn(x_v[0:16, :], _unpack(bqkv_p[1]))[0:1, :]
    v0 = _nn(x_v[0:16, :], _unpack(bqkv_p[2]))[0:1, :]
    for t in range(nt):
        k_scr[t, R:R + HALO, :] = jnp.broadcast_to(k0[:, t * LANES:(t + 1) * LANES], (HALO, LANES))
        v_scr[t, R:R + HALO, :] = jnp.broadcast_to(v0[:, t * LANES:(t + 1) * LANES], (HALO, LANES))

    def b_chunk(c, carry):
        r0 = pl.multiple_of(c * R, R)

        @pl.when(c + W_AHEAD < n_chunk)
        def _():
            w_start(c + W_AHEAD)

        for j in range(4):
            w_copy(c, j).wait()

        for t in range(nt):
            k_scr[t, 0:HALO, :] = k_scr[t, R:R + HALO, :]
            v_scr[t, 0:HALO, :] = v_scr[t, R:R + HALO, :]

        def project(i):
            xb = x_v[pl.ds(r0 + i * RS, RS), :]
            lo = HALO + i * RS
            kk = _nn(xb, _unpack(bqkv_p[1]))
            for t in range(nt):
                k_scr[t, lo:lo + RS, :] = kk[:, t * LANES:(t + 1) * LANES]
            vv = _nn(xb, _unpack(bqkv_p[2]))
            for t in range(nt):
                v_scr[t, lo:lo + RS, :] = vv[:, t * LANES:(t + 1) * LANES]
            q_scr[i * RS:(i + 1) * RS, :] = _nn(xb, _unpack(bqkv_p[0])) * b_scale
            g = jax.nn.sigmoid(jnp.sum(xb.astype(F32) * gate, axis=-1, keepdims=True))
            g_scr[pl.ds(r0 + i * RS, RS), :] = jnp.broadcast_to(g, (RS, LANES))

        def attend(i):
            for u in range(i * RS, (i + 1) * RS, RA):
                qs = [q_scr[u:u + RA, t * LANES:(t + 1) * LANES] for t in range(nt)]
                logits = []
                for w in range(B_WIN):
                    off = u + HALO - B_DIL * w
                    acc = qs[0] * k_scr[0, off:off + RA, :]
                    for t in range(1, nt):
                        acc = acc + qs[t] * k_scr[t, off:off + RA, :]
                    acc = acc + pltpu.roll(acc, 2 * B_HEADS, 1)
                    acc = acc + pltpu.roll(acc, B_HEADS, 1)
                    if u < B_DIL * w:
                        pos = r0 + u + jax.lax.broadcasted_iota(I32, (RA, LANES), 0)
                        acc = jnp.where(pos >= B_DIL * w, acc, NEG)
                    logits.append(acc)
                mx = functools.reduce(jnp.maximum, logits)
                es = [jnp.exp(l - mx) for l in logits]
                inv = 1.0 / functools.reduce(jnp.add, es)
                for t in range(nt):
                    acc = es[0] * v_scr[t, u + HALO:u + HALO + RA, :]
                    for w in range(1, B_WIN):
                        off = u + HALO - B_DIL * w
                        acc = acc + es[w] * v_scr[t, off:off + RA, :]
                    ob_scr[u // 2:(u + RA) // 2, t * LANES:(t + 1) * LANES] = _pack((acc * inv).astype(BF16))

        def mix(i):
            bb = _nn(_unpack(ob_scr[i * RS // 2:(i + 1) * RS // 2, :]), _unpack(bwo_p[...]))
            rows = pl.ds(r0 + i * RS, RS)
            b_scr[rows, :] = (1.0 - jnp.concatenate([g_scr[rows, :]] * nt, axis=1)) * bb

        def stage_weights(n):
            i, j = divmod(n, 4)
            p = c * ppc + i
            blk = stage[c, j, i * PW:(i + 1) * PW, :]
            if j < 3:
                wqkv_p[p, :, j * PW:(j + 1) * PW] = _pack(blk.T)
            else:
                wo_p[p] = _pack(blk)

        n_sub = R // RS
        todo = list(range(4 * ppc))
        for i in range(n_sub + 2):
            if i < n_sub:
                project(i)
            if 0 <= i - 2 < n_sub:
                mix(i - 2)
            if 0 <= i - 1 < n_sub:
                attend(i - 1)
            if i < n_sub:
                for _ in range(4 * ppc // n_sub):
                    stage_weights(todo.pop(0))
        assert not todo
        return carry

    jax.lax.fori_loop(0, n_chunk, b_chunk, 0)

    a_scale = Dh ** (-0.5)
    h_scr[0:M, :] = mem0_ref[...].astype(F32)

    def out_copy(i):
        rows = pl.ds(pl.multiple_of(i * (out_every * seg), out_every * seg), out_every * seg)
        return pltpu.make_async_copy(out_v.at[rows, :], out_hbm.at[rows, :], out_sem)

    def a_step(s, carry):
        r0 = pl.multiple_of(s * seg, seg)
        h_scr[M:L, :] = x_v[pl.ds(r0, seg), :].astype(F32)

        row = jax.lax.broadcasted_iota(I32, (L, 2 * L), 0)
        col = jax.lax.broadcasted_iota(I32, (L, 2 * L), 1)
        first = col < L
        key = jnp.where(first, col, col - L)
        visible = (row < M) | (row >= key)
        lane = jax.lax.broadcasted_iota(I32, (L, PW), 1)
        in_a = lane < Dh

        def block_diag(z):
            return jnp.concatenate([jnp.where(in_a, z, 0.0), jnp.where(in_a, 0.0, z)], axis=0).astype(BF16)

        def project(p):
            qkv = _nn(h_scr[...], _unpack(wqkv_p[p]))
            return qkv[:, 0:PW], block_diag(qkv[:, PW:2 * PW]), block_diag(qkv[:, 2 * PW:3 * PW])

        def probs(q, kbd):
            sc = jnp.where(visible, _nt(q, kbd) * a_scale, NEG)
            m_a = jnp.max(jnp.where(first, sc, -jnp.inf), axis=-1, keepdims=True)
            m_b = jnp.max(jnp.where(first, -jnp.inf, sc), axis=-1, keepdims=True)
            e = jnp.exp(sc - jnp.where(first, m_a, m_b))
            l_a = jnp.sum(jnp.where(first, e, 0.0), axis=-1, keepdims=True)
            l_b = jnp.sum(jnp.where(first, 0.0, e), axis=-1, keepdims=True)
            return e * jnp.where(first, 1.0 / l_a, 1.0 / l_b)

        def out_proj(p, acc):
            y = _nn(o_scr[:, p * PW:(p + 1) * PW], _unpack(wo_p[p]))
            return y if acc is None else acc + y

        qkv, pr, acc, n_out = {}, {}, None, 0
        for t in range(n_pair + 2):
            if t < n_pair:
                qkv[t] = project(t)
            else:
                for _ in range(3):
                    acc = out_proj(n_out, acc)
                    n_out += 1
            if 0 <= t - 1 < n_pair:
                pr[t - 1] = probs(qkv[t - 1][0], qkv[t - 1][1])
            if 0 <= t - 2 < n_pair:
                o_scr[:, (t - 2) * PW:(t - 1) * PW] = _nn(pr.pop(t - 2), qkv.pop(t - 2)[2])
        for p in range(n_out, n_pair):
            acc = out_proj(p, acc)

        h_scr[0:M, :] = acc[0:M, :]
        g = g_scr[pl.ds(r0, seg), :]
        g = jnp.concatenate([g] * nt, axis=1)
        out_v[pl.ds(r0, seg), :] = (g * acc[M:L, :] + b_scr[pl.ds(r0, seg), :]).astype(out_v.dtype)

        @pl.when(s % out_every == out_every - 1)
        def _():
            out_copy(s // out_every).start()

        return carry

    jax.lax.fori_loop(0, n_seg, a_step, 0)
    pltpu.make_async_copy(out_v, out_hbm, out_sem).wait()


@functools.partial(jax.jit, static_argnames=("A_seg_len",))
def pallas_gated_mix__memory_aug_recurrent_mem_tr__sliding_local_dilated__prompt_kernel(
    A_x: jax.Array,
    A_mem0: jax.Array,
    A_Wq: jax.Array,
    A_Wk: jax.Array,
    A_Wv: jax.Array,
    A_Wo: jax.Array,
    A_seg_len: int,
    B_x: jax.Array,
    B_wqkv: jax.Array,
    B_wo: jax.Array,
    gate_w: jax.Array,
):
    del B_x
    Bsz, S, D = A_x.shape
    _, H, Dh = A_Wq.shape
    M = A_mem0.shape[1]
    seg = int(A_seg_len)
    assert Bsz == 1 and S % seg == 0 and H % 2 == 0 and (2 * Dh) % LANES == 0 and D % LANES == 0
    n_chunk = 8
    out_every = 8
    n_pair = H // 2
    PW = 2 * Dh
    R = S // n_chunk
    L = M + seg

    def head_major(w):
        return jnp.transpose(w, (1, 2, 0)).reshape(H * Dh, D)

    any_spec = pl.BlockSpec(memory_space=pl.ANY)
    vmem_spec = pl.BlockSpec(memory_space=pltpu.VMEM)
    out = pl.pallas_call(
        functools.partial(_kernel, S=S, D=D, H=H, Dh=Dh, M=M, seg=seg,
                          n_chunk=n_chunk, out_every=out_every),
        out_shape=jax.ShapeDtypeStruct((S, D), A_x.dtype),
        in_specs=[any_spec, vmem_spec, any_spec, any_spec, any_spec, any_spec,
                  any_spec, any_spec, vmem_spec],
        out_specs=any_spec,
        scratch_shapes=[
            pltpu.VMEM((S, D), BF16),
            pltpu.VMEM((3, D, D), BF16),
            pltpu.VMEM((D, D), BF16),
            pltpu.VMEM((3, D // 2, D), I32),
            pltpu.VMEM((D // 2, D), I32),
            pltpu.VMEM((R, D), F32),
            pltpu.VMEM((D // LANES, HALO + R, LANES), F32),
            pltpu.VMEM((D // LANES, HALO + R, LANES), F32),
            pltpu.VMEM((R // 2, D), I32),
            pltpu.VMEM((S, LANES), F32),
            pltpu.VMEM((S, D), F32),
            pltpu.VMEM((n_chunk, 4, n_pair // n_chunk * PW, D), BF16),
            pltpu.VMEM((n_pair, D // 2, 3 * PW), I32),
            pltpu.VMEM((n_pair, PW // 2, D), I32),
            pltpu.VMEM((L, D), F32),
            pltpu.VMEM((L, H * Dh), F32),
            pltpu.VMEM((S, D), A_x.dtype),
            pltpu.SemaphoreType.DMA((5,)),
            pltpu.SemaphoreType.DMA((n_chunk, 4)),
            pltpu.SemaphoreType.DMA(()),
        ],
        compiler_params=pltpu.CompilerParams(vmem_limit_bytes=110 * 1024 * 1024),
    )(
        A_x.reshape(S, D),
        A_mem0.reshape(M, D),
        head_major(A_Wq),
        head_major(A_Wk),
        head_major(A_Wv),
        A_Wo.reshape(H * Dh, D),
        B_wqkv,
        B_wo,
        gate_w.reshape(1, D),
    )
    return out.reshape(Bsz, S, D)
```

```python
import functools

import jax
import jax.numpy as jnp
import jax.experimental.pallas as pl
import jax.experimental.pallas.tpu as pltpu

F32 = jnp.float32
BF16 = jnp.bfloat16
I32 = jnp.int32

LANES = 128
B_HEADS = 32
B_WIN = 8
B_DIL = 2
HALO = 16
NEG = -1000000000.0
RS = 64
RA = 16
A_UNROLL = 3
A_TAIL = 4
W_AHEAD = 3


def _nt(a, b):
    return jax.lax.dot_general(a, b, (((1,), (1,)), ((), ())), preferred_element_type=F32)


def _nn(a, b):
    return jax.lax.dot_general(a, b, (((1,), (0,)), ((), ())), preferred_element_type=F32)


def _pack(w):
    return pltpu.bitcast(w, I32)


def _unpack(w):
    return pltpu.bitcast(w, BF16)


def _kernel(x_hbm, mem0_ref, wq_hbm, wk_hbm, wv_hbm, wo_hbm, bqkv_hbm, bwo_hbm, gate_ref,
            out_hbm,
            x_v, bqkv_v, bwo_v, bwo_f, bqkv_p, bwo_p, q_scr, k_scr, v_scr, ob_scr, g_scr, b_scr,
            stage, wo_v, wqkv_p, wo_p, h_scr, o_scr, out_v,
            in_sem, w_sem, wo_sem, out_sem,
            *, S, D, H, Dh, M, seg, n_chunk):
    L = M + seg
    n_seg = S // seg
    n_pair = H // 2
    PW = 2 * Dh
    R = S // n_chunk
    ppc = n_pair // n_chunk
    nt = D // LANES
    dB = D // B_HEADS
    a_scale = Dh ** (-0.5)
    b_scale = dB ** (-0.5)

    def bqkv_copy(j):
        cols = pl.ds(j * D, D)
        return pltpu.make_async_copy(bqkv_hbm.at[:, cols], bqkv_v.at[j], in_sem.at[j])

    cp_x = pltpu.make_async_copy(x_hbm, x_v, in_sem.at[3])
    cp_bwo = pltpu.make_async_copy(bwo_hbm, bwo_v, in_sem.at[4])

    def chunk_rows(c):
        return pl.ds(pl.multiple_of(c * (ppc * PW), ppc * PW), ppc * PW)

    def w_copy(c, j):
        src = (wq_hbm, wk_hbm, wv_hbm)[j]
        return pltpu.make_async_copy(src.at[chunk_rows(c), :], stage.at[c, j], w_sem.at[c, j])

    def wo_copy(c):
        return pltpu.make_async_copy(wo_hbm.at[chunk_rows(c), :], wo_v.at[c], wo_sem.at[c])

    def w_start(c):
        for j in range(3):
            w_copy(c, j).start()

    def out_copy(row0, n):
        rows = pl.ds(row0, n)
        return pltpu.make_async_copy(out_v.at[rows, :], out_hbm.at[rows, :], out_sem)

    def block_diag(z):
        in_a = jax.lax.broadcasted_iota(I32, (L, PW), 1) < Dh
        return jnp.concatenate([jnp.where(in_a, z, 0.0), jnp.where(in_a, 0.0, z)], axis=0).astype(BF16)

    def a_project(p):
        qkv = _nn(h_scr[...], _unpack(wqkv_p[p]))
        return qkv[:, 0:PW], block_diag(qkv[:, PW:2 * PW]), block_diag(qkv[:, 2 * PW:3 * PW])

    def a_probs(q, kbd):
        row = jax.lax.broadcasted_iota(I32, (L, 2 * L), 0)
        col = jax.lax.broadcasted_iota(I32, (L, 2 * L), 1)
        first = col < L
        visible = (row < M) | (row >= jnp.where(first, col, col - L))
        sc = jnp.where(visible, _nt(q, kbd) * a_scale, NEG)
        m_a = jnp.max(jnp.where(first, sc, -jnp.inf), axis=-1, keepdims=True)
        m_b = jnp.max(jnp.where(first, -jnp.inf, sc), axis=-1, keepdims=True)
        e = jnp.exp(sc - jnp.where(first, m_a, m_b))
        l_a = jnp.sum(jnp.where(first, e, 0.0), axis=-1, keepdims=True)
        l_b = jnp.sum(jnp.where(first, 0.0, e), axis=-1, keepdims=True)
        return e * jnp.where(first, 1.0 / l_a, 1.0 / l_b)

    def a_out_proj(p, acc, lo, hi):
        y = _nn(o_scr[p], _unpack(wo_p[p, :, lo:hi]))
        return y if acc is None else acc + y

    def a_finish(r0, acc, p0):
        g = g_scr[pl.ds(r0, seg), :]
        for lo, hi in ((0, D - LANES), (D - LANES, D)):
            part = acc[:, lo:hi]
            for p in range(p0, n_pair):
                part = a_out_proj(p, part, lo, hi)
            h_scr[0:M, lo:hi] = part[0:M, :]
            gg = jnp.concatenate([g] * ((hi - lo) // LANES), axis=1)
            out_v[pl.ds(r0, seg), lo:hi] = (gg * part[M:L, :] + b_scr[pl.ds(r0, seg), lo:hi]).astype(out_v.dtype)

    bqkv_copy(0).start()

    ri = jax.lax.broadcasted_iota(I32, (D, D), 0)
    ci = jax.lax.broadcasted_iota(I32, (D, D), 1)
    perm = jnp.where(ri == (ci % B_HEADS) * dB + ci // B_HEADS, 1.0, 0.0).astype(BF16)
    bqkv_copy(0).wait()
    bqkv_copy(1).start()
    bqkv_copy(2).start()
    cp_bwo.start()
    cp_x.start()
    bqkv_p[0] = _pack(_nn(bqkv_v[0], perm).astype(BF16))
    bqkv_copy(1).wait()
    w_start(0)
    bqkv_p[1] = _pack(_nn(bqkv_v[1], perm).astype(BF16))
    bqkv_copy(2).wait()
    w_start(1)
    cp_bwo.wait()
    bqkv_p[2] = _pack(_nn(bqkv_v[2], perm).astype(BF16))
    for t in range(nt):
        bwo_f[t] = bwo_v[:, t * LANES:(t + 1) * LANES].astype(F32)
    for t in range(nt):
        for d in range(dB):
            rows = bwo_f[t, pl.ds(d, B_HEADS, stride=dB), :]
            bwo_p[d * B_HEADS // 2:(d + 1) * B_HEADS // 2, t * LANES:(t + 1) * LANES] = _pack(rows.astype(BF16))
    cp_x.wait()
    w_start(2)

    gate = gate_ref[...].astype(F32)
    h_scr[0:M, :] = mem0_ref[...].astype(F32)
    h_scr[M:L, :] = x_v[0:seg, :].astype(F32)

    k0 = _nn(x_v[0:16, :], _unpack(bqkv_p[1]))[0:1, :]
    v0 = _nn(x_v[0:16, :], _unpack(bqkv_p[2]))[0:1, :]
    for t in range(nt):
        k_scr[t, R:R + HALO, :] = jnp.broadcast_to(k0[:, t * LANES:(t + 1) * LANES], (HALO, LANES))
        v_scr[t, R:R + HALO, :] = jnp.broadcast_to(v0[:, t * LANES:(t + 1) * LANES], (HALO, LANES))

    def b_chunk(c, carry):
        r0 = pl.multiple_of(c * R, R)

        @pl.when(c + W_AHEAD < n_chunk)
        def _():
            w_start(c + W_AHEAD)

        @pl.when(c >= n_chunk // 2)
        def _():
            wo_copy(2 * c - n_chunk).start()
            wo_copy(2 * c - n_chunk + 1).start()

        for j in range(3):
            w_copy(c, j).wait()

        for t in range(nt):
            k_scr[t, 0:HALO, :] = k_scr[t, R:R + HALO, :]
            v_scr[t, 0:HALO, :] = v_scr[t, R:R + HALO, :]

        def project(i):
            xb = x_v[pl.ds(r0 + i * RS, RS), :]
            lo = HALO + i * RS
            kk = _nn(xb, _unpack(bqkv_p[1]))
            for t in range(nt):
                k_scr[t, lo:lo + RS, :] = kk[:, t * LANES:(t + 1) * LANES]
            vv = _nn(xb, _unpack(bqkv_p[2]))
            for t in range(nt):
                v_scr[t, lo:lo + RS, :] = vv[:, t * LANES:(t + 1) * LANES]
            q_scr[i * RS:(i + 1) * RS, :] = _nn(xb, _unpack(bqkv_p[0])) * b_scale
            g = jax.nn.sigmoid(jnp.sum(xb.astype(F32) * gate, axis=-1, keepdims=True))
            g_scr[pl.ds(r0 + i * RS, RS), :] = jnp.broadcast_to(g, (RS, LANES))

        def attend(i):
            for u in range(i * RS, (i + 1) * RS, RA):
                qs = [q_scr[u:u + RA, t * LANES:(t + 1) * LANES] for t in range(nt)]
                logits = []
                for w in range(B_WIN):
                    off = u + HALO - B_DIL * w
                    acc = qs[0] * k_scr[0, off:off + RA, :]
                    for t in range(1, nt):
                        acc = acc + qs[t] * k_scr[t, off:off + RA, :]
                    acc = acc + pltpu.roll(acc, 2 * B_HEADS, 1)
                    acc = acc + pltpu.roll(acc, B_HEADS, 1)
                    if u < B_DIL * w:
                        pos = r0 + u + jax.lax.broadcasted_iota(I32, (RA, LANES), 0)
                        acc = jnp.where(pos >= B_DIL * w, acc, NEG)
                    logits.append(acc)
                mx = functools.reduce(jnp.maximum, logits)
                es = [jnp.exp(l - mx) for l in logits]
                inv = 1.0 / functools.reduce(jnp.add, es)
                for t in range(nt):
                    acc = es[0] * v_scr[t, u + HALO:u + HALO + RA, :]
                    for w in range(1, B_WIN):
                        off = u + HALO - B_DIL * w
                        acc = acc + es[w] * v_scr[t, off:off + RA, :]
                    ob_scr[u // 2:(u + RA) // 2, t * LANES:(t + 1) * LANES] = _pack((acc * inv).astype(BF16))

        def mix(i):
            bb = _nn(_unpack(ob_scr[i * RS // 2:(i + 1) * RS // 2, :]), _unpack(bwo_p[...]))
            rows = pl.ds(r0 + i * RS, RS)
            b_scr[rows, :] = (1.0 - jnp.concatenate([g_scr[rows, :]] * nt, axis=1)) * bb

        def stage_pair(i):
            for j in range(3):
                wqkv_p[c * ppc + i, :, j * PW:(j + 1) * PW] = _pack(stage[c, j, i * PW:(i + 1) * PW, :].T)

        n_sub = R // RS
        assert ppc + 2 <= n_sub + 1
        qkv, pr = {}, {}
        for i in range(n_sub + 2):
            if i < ppc:
                stage_pair(i)
            if 0 <= i - 2 < ppc:
                pr[i - 2] = a_probs(qkv[i - 2][0], qkv[i - 2][1])
            if i < n_sub:
                project(i)
            if 0 <= i - 2 < n_sub:
                mix(i - 2)
            if 0 <= i - 3 < ppc:
                o_scr[c * ppc + i - 3] = _nn(pr[i - 3], qkv[i - 3][2])
            if 0 <= i - 1 < ppc:
                qkv[i - 1] = a_project(c * ppc + i - 1)
            if 0 <= i - 1 < n_sub:
                attend(i - 1)
        return carry

    jax.lax.fori_loop(0, n_chunk, b_chunk, 0)

    for c in range(n_chunk):
        wo_copy(c).wait()
    acc0 = None
    for p in range(n_pair):
        c, i = divmod(p, ppc)
        wo_p[p] = _pack(wo_v[c, i * PW:(i + 1) * PW, :])
        if p >= A_TAIL:
            acc0 = a_out_proj(p - A_TAIL, acc0, 0, D)
    a_finish(0, acc0, n_pair - A_TAIL)
    out_copy(0, seg).start()

    def a_step(s):
        r0 = pl.multiple_of(s * seg, seg)
        h_scr[M:L, :] = x_v[pl.ds(r0, seg), :].astype(F32)

        qkv, pr, acc, n_out = {}, {}, None, 0
        for t in range(n_pair + 2):
            if t < n_pair:
                qkv[t] = a_project(t)
            else:
                for _ in range(3):
                    acc = a_out_proj(n_out, acc, 0, D)
                    n_out += 1
            if 0 <= t - 1 < n_pair:
                pr[t - 1] = a_probs(qkv[t - 1][0], qkv[t - 1][1])
            if 0 <= t - 2 < n_pair:
                o_scr[t - 2] = _nn(pr.pop(t - 2), qkv.pop(t - 2)[2])
        for p in range(n_out, n_pair - A_TAIL):
            acc = a_out_proj(p, acc, 0, D)
        a_finish(r0, acc, n_pair - A_TAIL)

    def a_body(i, carry):
        s0 = 1 + i * A_UNROLL
        for u in range(A_UNROLL):
            a_step(s0 + u)
        out_copy(pl.multiple_of(s0 * seg, seg), A_UNROLL * seg).start()
        return carry

    assert (n_seg - 1) % A_UNROLL == 0
    jax.lax.fori_loop(0, (n_seg - 1) // A_UNROLL, a_body, 0)
    pltpu.make_async_copy(out_v, out_hbm, out_sem).wait()


@functools.partial(jax.jit, static_argnames=("A_seg_len",))
def pallas_gated_mix__memory_aug_recurrent_mem_tr__sliding_local_dilated__prompt_kernel(
    A_x: jax.Array,
    A_mem0: jax.Array,
    A_Wq: jax.Array,
    A_Wk: jax.Array,
    A_Wv: jax.Array,
    A_Wo: jax.Array,
    A_seg_len: int,
    B_x: jax.Array,
    B_wqkv: jax.Array,
    B_wo: jax.Array,
    gate_w: jax.Array,
):
    del B_x
    Bsz, S, D = A_x.shape
    _, H, Dh = A_Wq.shape
    M = A_mem0.shape[1]
    seg = int(A_seg_len)
    assert Bsz == 1 and S % seg == 0 and H % 2 == 0 and (2 * Dh) % LANES == 0 and D % LANES == 0
    n_chunk = 8
    n_pair = H // 2
    PW = 2 * Dh
    R = S // n_chunk
    L = M + seg

    def head_major(w):
        return jnp.transpose(w, (1, 2, 0)).reshape(H * Dh, D)

    any_spec = pl.BlockSpec(memory_space=pl.ANY)
    vmem_spec = pl.BlockSpec(memory_space=pltpu.VMEM)
    out = pl.pallas_call(
        functools.partial(_kernel, S=S, D=D, H=H, Dh=Dh, M=M, seg=seg,
                          n_chunk=n_chunk),
        out_shape=jax.ShapeDtypeStruct((S, D), A_x.dtype),
        in_specs=[any_spec, vmem_spec, any_spec, any_spec, any_spec, any_spec,
                  any_spec, any_spec, vmem_spec],
        out_specs=any_spec,
        scratch_shapes=[
            pltpu.VMEM((S, D), BF16),
            pltpu.VMEM((3, D, D), BF16),
            pltpu.VMEM((D, D), BF16),
            pltpu.VMEM((D // LANES, D, LANES), F32),
            pltpu.VMEM((3, D // 2, D), I32),
            pltpu.VMEM((D // 2, D), I32),
            pltpu.VMEM((R, D), F32),
            pltpu.VMEM((D // LANES, HALO + R, LANES), F32),
            pltpu.VMEM((D // LANES, HALO + R, LANES), F32),
            pltpu.VMEM((R // 2, D), I32),
            pltpu.VMEM((S, LANES), F32),
            pltpu.VMEM((S, D), F32),
            pltpu.VMEM((n_chunk, 3, n_pair // n_chunk * PW, D), BF16),
            pltpu.VMEM((n_chunk, n_pair // n_chunk * PW, D), BF16),
            pltpu.VMEM((n_pair, D // 2, 3 * PW), I32),
            pltpu.VMEM((n_pair, PW // 2, D), I32),
            pltpu.VMEM((L, D), F32),
            pltpu.VMEM((n_pair, L, PW), F32),
            pltpu.VMEM((S, D), A_x.dtype),
            pltpu.SemaphoreType.DMA((5,)),
            pltpu.SemaphoreType.DMA((n_chunk, 3)),
            pltpu.SemaphoreType.DMA((n_chunk,)),
            pltpu.SemaphoreType.DMA(()),
        ],
        compiler_params=pltpu.CompilerParams(vmem_limit_bytes=110 * 1024 * 1024),
    )(
        A_x.reshape(S, D),
        A_mem0.reshape(M, D),
        head_major(A_Wq),
        head_major(A_Wk),
        head_major(A_Wv),
        A_Wo.reshape(H * Dh, D),
        B_wqkv,
        B_wo,
        gate_w.reshape(1, D),
    )
    return out.reshape(Bsz, S, D)
```

```python
import functools

import jax
import jax.numpy as jnp
import jax.experimental.pallas as pl
import jax.experimental.pallas.tpu as pltpu

F32 = jnp.float32
BF16 = jnp.bfloat16
I32 = jnp.int32

LANES = 128
B_HEADS = 32
B_WIN = 8
B_DIL = 2
HALO = 16
NEG = -1000000000.0
RS = 64
RA = 16
A_UNROLL = 3
A_TAIL = 4
B_ORDER = "T0 p0 p1 a0 T1 p2 a1 p3 a2 Q0 Q1 a3 S0 m0 m1 S1 m2 V0 m3 V1"
B_ORDER_FIRST = "p0 p1 a0 p2 a1 p3 a2 m0 a3 m1 m2 m3"
LAST_ORDER = "T0 O0 O1 O2 O3 O4 O5 T1 Q0 O6 O7 S0 Q1 O8 S1 O9 V0 O10 O11 V1 O12 O13"


def _nt(a, b):
    return jax.lax.dot_general(a, b, (((1,), (1,)), ((), ())), preferred_element_type=F32)


def _nn(a, b):
    return jax.lax.dot_general(a, b, (((1,), (0,)), ((), ())), preferred_element_type=F32)


def _pack(w):
    return pltpu.bitcast(w, I32)


def _unpack(w):
    return pltpu.bitcast(w, BF16)


def _kernel(x_hbm, mem0_ref, wq_hbm, wk_hbm, wv_hbm, wo_hbm, bqkv_hbm, bwo_hbm, gate_ref,
            out_hbm,
            x_v, bqkv_v, bwo_v, perm_f, bqkv_p, bwo_p, q_scr, k_scr, v_scr, ob_scr, g_scr, b_scr,
            stage, wo_v, wqkv_p, wo_p, h_scr, o_scr, out_v,
            in_sem, w_sem, wo_sem, out_sem,
            *, S, D, H, Dh, M, seg, n_chunk):
    L = M + seg
    n_seg = S // seg
    n_pair = H // 2
    PW = 2 * Dh
    R = S // n_chunk
    ppc = n_pair // n_chunk
    nt = D // LANES
    dB = D // B_HEADS
    a_scale = Dh ** (-0.5)
    b_scale = dB ** (-0.5)

    def bqkv_copy(j):
        cols = pl.ds(j * D, D)
        return pltpu.make_async_copy(bqkv_hbm.at[:, cols], bqkv_v.at[j], in_sem.at[j])

    cp_bwo = pltpu.make_async_copy(bwo_hbm, bwo_v, in_sem.at[3])

    def x_copy(part):
        rows = (pl.ds(0, R), pl.ds(R, S - R))[part]
        return pltpu.make_async_copy(x_hbm.at[rows, :], x_v.at[rows, :], in_sem.at[4 + part])

    def chunk_rows(c):
        return pl.ds(pl.multiple_of(c * (ppc * PW), ppc * PW), ppc * PW)

    def w_copy(c, j):
        src = (wq_hbm, wk_hbm, wv_hbm)[j]
        return pltpu.make_async_copy(src.at[chunk_rows(c), :], stage.at[c, j], w_sem.at[c, j])

    def wo_copy(c):
        return pltpu.make_async_copy(wo_hbm.at[chunk_rows(c), :], wo_v.at[c], wo_sem.at[c])

    def w_start(c):
        for j in range(3):
            w_copy(c, j).start()

    def out_copy(row0, n):
        rows = pl.ds(row0, n)
        return pltpu.make_async_copy(out_v.at[rows, :], out_hbm.at[rows, :], out_sem)

    def block_diag(z):
        in_a = jax.lax.broadcasted_iota(I32, (L, PW), 1) < Dh
        return jnp.concatenate([jnp.where(in_a, z, 0.0), jnp.where(in_a, 0.0, z)], axis=0).astype(BF16)

    def a_project(p):
        qkv = _nn(h_scr[...], _unpack(wqkv_p[p]))
        return qkv[:, 0:PW], block_diag(qkv[:, PW:2 * PW]), block_diag(qkv[:, 2 * PW:3 * PW])

    def a_probs(q, kbd):
        row = jax.lax.broadcasted_iota(I32, (L, 2 * L), 0)
        col = jax.lax.broadcasted_iota(I32, (L, 2 * L), 1)
        first = col < L
        visible = (row < M) | (row >= jnp.where(first, col, col - L))
        sc = jnp.where(visible, _nt(q, kbd) * a_scale, NEG)
        m_a = jnp.max(jnp.where(first, sc, -jnp.inf), axis=-1, keepdims=True)
        m_b = jnp.max(jnp.where(first, -jnp.inf, sc), axis=-1, keepdims=True)
        e = jnp.exp(sc - jnp.where(first, m_a, m_b))
        l_a = jnp.sum(jnp.where(first, e, 0.0), axis=-1, keepdims=True)
        l_b = jnp.sum(jnp.where(first, 0.0, e), axis=-1, keepdims=True)
        return e * jnp.where(first, 1.0 / l_a, 1.0 / l_b)

    def a_out_proj(p, acc, lo, hi):
        y = _nn(o_scr[p], _unpack(wo_p[p, :, lo:hi]))
        return y if acc is None else acc + y

    def a_finish(r0, acc, p0):
        g = g_scr[pl.ds(r0, seg), :]
        for lo, hi in ((0, D - LANES), (D - LANES, D)):
            part = acc[:, lo:hi]
            for p in range(p0, n_pair):
                part = a_out_proj(p, part, lo, hi)
            h_scr[0:M, lo:hi] = part[0:M, :]
            gg = jnp.concatenate([g] * ((hi - lo) // LANES), axis=1)
            out_v[pl.ds(r0, seg), lo:hi] = (gg * part[M:L, :] + b_scr[pl.ds(r0, seg), lo:hi]).astype(out_v.dtype)

    bqkv_copy(1).start()
    bqkv_copy(2).start()

    def reorder_rows(w, j):
        for t in range(nt):
            perm_f[j, t] = w[:, t * LANES:(t + 1) * LANES].astype(F32)
        return jnp.concatenate(
            [jnp.concatenate([perm_f[j, t, pl.ds(d, B_HEADS, stride=dB), :] for d in range(dB)], axis=0)
             for t in range(nt)], axis=1).astype(BF16)

    bqkv_copy(1).wait()
    bqkv_copy(0).start()
    x_copy(0).start()
    bqkv_p[1] = _pack(reorder_rows(bqkv_v[1].T, 1).T)
    bqkv_copy(2).wait()
    cp_bwo.start()
    x_copy(1).start()
    bqkv_p[2] = _pack(reorder_rows(bqkv_v[2].T, 2).T)
    bqkv_copy(0).wait()
    w_start(0)
    bqkv_p[0] = _pack(reorder_rows(bqkv_v[0].T, 0).T)
    cp_bwo.wait()
    x_copy(0).wait()
    bwo_p[...] = _pack(reorder_rows(bwo_v[...], 3))

    gate = gate_ref[...].astype(F32)
    h_scr[0:M, :] = mem0_ref[...].astype(F32)
    h_scr[M:L, :] = x_v[0:seg, :].astype(F32)

    k0 = _nn(x_v[0:16, :], _unpack(bqkv_p[1]))[0:1, :]
    v0 = _nn(x_v[0:16, :], _unpack(bqkv_p[2]))[0:1, :]
    for t in range(nt):
        k_scr[t, R:R + HALO, :] = jnp.broadcast_to(k0[:, t * LANES:(t + 1) * LANES], (HALO, LANES))
        v_scr[t, R:R + HALO, :] = jnp.broadcast_to(v0[:, t * LANES:(t + 1) * LANES], (HALO, LANES))

    def stage_pair(c, i):
        for j in range(3):
            wqkv_p[c * ppc + i, :, j * PW:(j + 1) * PW] = _pack(stage[c, j, i * PW:(i + 1) * PW, :].T)

    def a_first(c, kind, i, qkv, pr):
        if kind == "T":
            stage_pair(c, i)
        elif kind == "Q":
            qkv[i] = a_project(c * ppc + i)
        elif kind == "S":
            pr[i] = a_probs(qkv[i][0], qkv[i][1])
        else:
            o_scr[c * ppc + i] = _nn(pr[i], qkv[i][2])

    def b_chunk(c, order):
        r0 = pl.multiple_of(c * R, R)
        for t in range(nt):
            k_scr[t, 0:HALO, :] = k_scr[t, R:R + HALO, :]
            v_scr[t, 0:HALO, :] = v_scr[t, R:R + HALO, :]

        def project(i):
            xb = x_v[pl.ds(r0 + i * RS, RS), :]
            lo = HALO + i * RS
            kk = _nn(xb, _unpack(bqkv_p[1]))
            for t in range(nt):
                k_scr[t, lo:lo + RS, :] = kk[:, t * LANES:(t + 1) * LANES]
            vv = _nn(xb, _unpack(bqkv_p[2]))
            for t in range(nt):
                v_scr[t, lo:lo + RS, :] = vv[:, t * LANES:(t + 1) * LANES]
            q_scr[i * RS:(i + 1) * RS, :] = _nn(xb, _unpack(bqkv_p[0])) * b_scale
            g = jax.nn.sigmoid(jnp.sum(xb.astype(F32) * gate, axis=-1, keepdims=True))
            g_scr[pl.ds(r0 + i * RS, RS), :] = jnp.broadcast_to(g, (RS, LANES))

        def attend(i):
            for u in range(i * RS, (i + 1) * RS, RA):
                qs = [q_scr[u:u + RA, t * LANES:(t + 1) * LANES] for t in range(nt)]
                logits = []
                for w in range(B_WIN):
                    off = u + HALO - B_DIL * w
                    acc = qs[0] * k_scr[0, off:off + RA, :]
                    for t in range(1, nt):
                        acc = acc + qs[t] * k_scr[t, off:off + RA, :]
                    acc = acc + pltpu.roll(acc, 2 * B_HEADS, 1)
                    acc = acc + pltpu.roll(acc, B_HEADS, 1)
                    if u < B_DIL * w:
                        pos = r0 + u + jax.lax.broadcasted_iota(I32, (RA, LANES), 0)
                        acc = jnp.where(pos >= B_DIL * w, acc, NEG)
                    logits.append(acc)
                mx = functools.reduce(jnp.maximum, logits)
                es = [jnp.exp(l - mx) for l in logits]
                inv = 1.0 / functools.reduce(jnp.add, es)
                for t in range(nt):
                    acc = es[0] * v_scr[t, u + HALO:u + HALO + RA, :]
                    for w in range(1, B_WIN):
                        off = u + HALO - B_DIL * w
                        acc = acc + es[w] * v_scr[t, off:off + RA, :]
                    ob_scr[u // 2:(u + RA) // 2, t * LANES:(t + 1) * LANES] = _pack((acc * inv).astype(BF16))

        def mix(i):
            bb = _nn(_unpack(ob_scr[i * RS // 2:(i + 1) * RS // 2, :]), _unpack(bwo_p[...]))
            rows = pl.ds(r0 + i * RS, RS)
            b_scr[rows, :] = (1.0 - jnp.concatenate([g_scr[rows, :]] * nt, axis=1)) * bb

        qkv, pr = {}, {}
        for op in order.split():
            kind, i = op[0], int(op[1:])
            if kind in "pam":
                {"p": project, "a": attend, "m": mix}[kind](i)
            else:
                a_first(c - 1, kind, i, qkv, pr)

    w_start(1)
    wo_copy(0).start()
    b_chunk(0, B_ORDER_FIRST)
    x_copy(1).wait()

    def b_body(c, carry):
        @pl.when(c + 1 < n_chunk)
        def _():
            w_start(c + 1)

        wo_copy(c).start()
        for j in range(3):
            w_copy(c - 1, j).wait()
        b_chunk(c, B_ORDER)
        return carry

    jax.lax.fori_loop(1, n_chunk, b_body, 0)

    for j in range(3):
        w_copy(n_chunk - 1, j).wait()
    for c in range(n_chunk):
        wo_copy(c).wait()

    def repack_wo(p):
        c, i = divmod(p, ppc)
        wo_p[p] = _pack(wo_v[c, i * PW:(i + 1) * PW, :])

    qkv0, pr0, acc0 = {}, {}, None
    repack_wo(0)
    for op in LAST_ORDER.split():
        kind, i = op[0], int(op[1:])
        if kind == "O":
            repack_wo(i + 1)
            acc0 = a_out_proj(i, acc0, 0, D)
        else:
            a_first(n_chunk - 1, kind, i, qkv0, pr0)
    repack_wo(n_pair - 1)
    a_finish(0, acc0, n_pair - ppc)
    out_copy(0, seg).start()

    def a_step(s):
        r0 = pl.multiple_of(s * seg, seg)
        h_scr[M:L, :] = x_v[pl.ds(r0, seg), :].astype(F32)

        qkv, pr, acc, n_out = {}, {}, None, 0
        for t in range(n_pair + 2):
            if t < n_pair:
                qkv[t] = a_project(t)
            else:
                for _ in range(3):
                    acc = a_out_proj(n_out, acc, 0, D)
                    n_out += 1
            if 0 <= t - 1 < n_pair:
                pr[t - 1] = a_probs(qkv[t - 1][0], qkv[t - 1][1])
            if 0 <= t - 2 < n_pair:
                o_scr[t - 2] = _nn(pr.pop(t - 2), qkv.pop(t - 2)[2])
        for p in range(n_out, n_pair - A_TAIL):
            acc = a_out_proj(p, acc, 0, D)
        a_finish(r0, acc, n_pair - A_TAIL)

    def a_body(i, carry):
        s0 = 1 + i * A_UNROLL
        for u in range(A_UNROLL):
            a_step(s0 + u)
        out_copy(pl.multiple_of(s0 * seg, seg), A_UNROLL * seg).start()
        return carry

    assert (n_seg - 1) % A_UNROLL == 0
    jax.lax.fori_loop(0, (n_seg - 1) // A_UNROLL, a_body, 0)
    pltpu.make_async_copy(out_v, out_hbm, out_sem).wait()


@functools.partial(jax.jit, static_argnames=("A_seg_len",))
def pallas_gated_mix__memory_aug_recurrent_mem_tr__sliding_local_dilated__prompt_kernel(
    A_x: jax.Array,
    A_mem0: jax.Array,
    A_Wq: jax.Array,
    A_Wk: jax.Array,
    A_Wv: jax.Array,
    A_Wo: jax.Array,
    A_seg_len: int,
    B_x: jax.Array,
    B_wqkv: jax.Array,
    B_wo: jax.Array,
    gate_w: jax.Array,
):
    del B_x
    Bsz, S, D = A_x.shape
    _, H, Dh = A_Wq.shape
    M = A_mem0.shape[1]
    seg = int(A_seg_len)
    assert Bsz == 1 and S % seg == 0 and H % 2 == 0 and (2 * Dh) % LANES == 0 and D % LANES == 0
    n_chunk = 8
    n_pair = H // 2
    PW = 2 * Dh
    R = S // n_chunk
    L = M + seg

    def head_major(w):
        return jnp.transpose(w, (1, 2, 0)).reshape(H * Dh, D)

    any_spec = pl.BlockSpec(memory_space=pl.ANY)
    vmem_spec = pl.BlockSpec(memory_space=pltpu.VMEM)
    out = pl.pallas_call(
        functools.partial(_kernel, S=S, D=D, H=H, Dh=Dh, M=M, seg=seg,
                          n_chunk=n_chunk),
        out_shape=jax.ShapeDtypeStruct((S, D), A_x.dtype),
        in_specs=[any_spec, vmem_spec, any_spec, any_spec, any_spec, any_spec,
                  any_spec, any_spec, vmem_spec],
        out_specs=any_spec,
        scratch_shapes=[
            pltpu.VMEM((S, D), BF16),
            pltpu.VMEM((3, D, D), BF16),
            pltpu.VMEM((D, D), BF16),
            pltpu.VMEM((4, D // LANES, D, LANES), F32),
            pltpu.VMEM((3, D // 2, D), I32),
            pltpu.VMEM((D // 2, D), I32),
            pltpu.VMEM((R, D), F32),
            pltpu.VMEM((D // LANES, HALO + R, LANES), F32),
            pltpu.VMEM((D // LANES, HALO + R, LANES), F32),
            pltpu.VMEM((R // 2, D), I32),
            pltpu.VMEM((S, LANES), F32),
            pltpu.VMEM((S, D), F32),
            pltpu.VMEM((n_chunk, 3, n_pair // n_chunk * PW, D), BF16),
            pltpu.VMEM((n_chunk, n_pair // n_chunk * PW, D), BF16),
            pltpu.VMEM((n_pair, D // 2, 3 * PW), I32),
            pltpu.VMEM((n_pair, PW // 2, D), I32),
            pltpu.VMEM((L, D), F32),
            pltpu.VMEM((n_pair, L, PW), F32),
            pltpu.VMEM((S, D), A_x.dtype),
            pltpu.SemaphoreType.DMA((6,)),
            pltpu.SemaphoreType.DMA((n_chunk, 3)),
            pltpu.SemaphoreType.DMA((n_chunk,)),
            pltpu.SemaphoreType.DMA(()),
        ],
        compiler_params=pltpu.CompilerParams(vmem_limit_bytes=110 * 1024 * 1024),
    )(
        A_x.reshape(S, D),
        A_mem0.reshape(M, D),
        head_major(A_Wq),
        head_major(A_Wk),
        head_major(A_Wv),
        A_Wo.reshape(H * Dh, D),
        B_wqkv,
        B_wo,
        gate_w.reshape(1, D),
    )
    return out.reshape(Bsz, S, D)
```

```python
import functools

import jax
import jax.numpy as jnp
import jax.experimental.pallas as pl
import jax.experimental.pallas.tpu as pltpu

F32 = jnp.float32
BF16 = jnp.bfloat16
I32 = jnp.int32

LANES = 128
B_HEADS = 32
B_WIN = 8
B_DIL = 2
HALO = 16
NEG = -1000000000.0
RS = 64
RA = 16
A_UNROLL = 3
A_TAIL = 4
B_ORDER = "T0 p0 p1 a0 T1 p2 a1 p3 a2 Q0 Q1 a3 S0 m0 m1 S1 m2 V0 m3 V1"
B_ORDER_FIRST = "q0 q1 a0 q2 a1 q3 w1 a2 m0 a3 m1 m2 m3"
LAST_ORDER = "T0 O0 O1 O2 O3 O4 O5 T1 Q0 O6 O7 S0 Q1 O8 S1 O9 V0 O10 V1 O11 O12 O13"
WO_ISSUE = (1, 2, 3, 4, 5, 6, 7, 7)


def _nt(a, b):
    return jax.lax.dot_general(a, b, (((1,), (1,)), ((), ())), preferred_element_type=F32)


def _nn(a, b):
    return jax.lax.dot_general(a, b, (((1,), (0,)), ((), ())), preferred_element_type=F32)


def _pack(w):
    return pltpu.bitcast(w, I32)


def _unpack(w):
    return pltpu.bitcast(w, BF16)


def _kernel(x_hbm, mem0_ref, wq_hbm, wk_hbm, wv_hbm, wo_hbm, bqkv_hbm, bwo_hbm, gate_ref,
            out_hbm,
            x_v, bqkv_v, bwo_v, perm_f, bqkv_p, bwo_p, q_scr, k_scr, v_scr, ob_scr, g_scr, b_scr,
            stage, wo_v, wqkv_p, wo_p, h_scr, o_scr, out_v,
            in_sem, x_sem, w_sem, wo_sem, out_sem,
            *, S, D, H, Dh, M, seg, n_chunk):
    L = M + seg
    n_seg = S // seg
    n_pair = H // 2
    PW = 2 * Dh
    R = S // n_chunk
    ppc = n_pair // n_chunk
    nt = D // LANES
    dB = D // B_HEADS
    a_scale = Dh ** (-0.5)
    b_scale = dB ** (-0.5)

    def bqkv_copy(j):
        cols = pl.ds(j * D, D)
        return pltpu.make_async_copy(bqkv_hbm.at[:, cols], bqkv_v.at[j], in_sem.at[j])

    cp_bwo = pltpu.make_async_copy(bwo_hbm, bwo_v, in_sem.at[3])

    def x_copy(c):
        rows = pl.ds(pl.multiple_of(c * R, R), R)
        return pltpu.make_async_copy(x_hbm.at[rows, :], x_v.at[rows, :], x_sem.at[c])

    def chunk_rows(c):
        return pl.ds(pl.multiple_of(c * (ppc * PW), ppc * PW), ppc * PW)

    def w_copy(c, j):
        src = (wq_hbm, wk_hbm, wv_hbm)[j]
        return pltpu.make_async_copy(src.at[chunk_rows(c), :], stage.at[c, j], w_sem.at[c, j])

    def wo_copy(c):
        return pltpu.make_async_copy(wo_hbm.at[chunk_rows(c), :], wo_v.at[c], wo_sem.at[c])

    def w_start(c):
        for j in range(3):
            w_copy(c, j).start()

    def out_copy(row0, n):
        rows = pl.ds(row0, n)
        return pltpu.make_async_copy(out_v.at[rows, :], out_hbm.at[rows, :], out_sem)

    def block_diag(z):
        in_a = jax.lax.broadcasted_iota(I32, (L, PW), 1) < Dh
        return jnp.concatenate([jnp.where(in_a, z, 0.0), jnp.where(in_a, 0.0, z)], axis=0).astype(BF16)

    def a_project(p):
        qkv = _nn(h_scr[...], _unpack(wqkv_p[p]))
        return qkv[:, 0:PW], block_diag(qkv[:, PW:2 * PW]), block_diag(qkv[:, 2 * PW:3 * PW])

    def a_probs(q, kbd):
        row = jax.lax.broadcasted_iota(I32, (L, 2 * L), 0)
        col = jax.lax.broadcasted_iota(I32, (L, 2 * L), 1)
        first = col < L
        visible = (row < M) | (row >= jnp.where(first, col, col - L))
        sc = jnp.where(visible, _nt(q, kbd) * a_scale, NEG)
        m_a = jnp.max(jnp.where(first, sc, -jnp.inf), axis=-1, keepdims=True)
        m_b = jnp.max(jnp.where(first, -jnp.inf, sc), axis=-1, keepdims=True)
        e = jnp.exp(sc - jnp.where(first, m_a, m_b))
        l_a = jnp.sum(jnp.where(first, e, 0.0), axis=-1, keepdims=True)
        l_b = jnp.sum(jnp.where(first, 0.0, e), axis=-1, keepdims=True)
        return e * jnp.where(first, 1.0 / l_a, 1.0 / l_b)

    def a_out_proj(p, acc, lo, hi):
        y = _nn(o_scr[p], _unpack(wo_p[p, :, lo:hi]))
        return y if acc is None else acc + y

    def a_finish(r0, acc, p0):
        g = g_scr[pl.ds(r0, seg), :]
        for lo, hi in ((0, D - LANES), (D - LANES, D)):
            part = acc[:, lo:hi]
            for p in range(p0, n_pair):
                part = a_out_proj(p, part, lo, hi)
            h_scr[0:M, lo:hi] = part[0:M, :]
            gg = jnp.concatenate([g] * ((hi - lo) // LANES), axis=1)
            out_v[pl.ds(r0, seg), lo:hi] = (gg * part[M:L, :] + b_scr[pl.ds(r0, seg), lo:hi]).astype(out_v.dtype)

    bqkv_copy(1).start()
    x_copy(0).start()

    def reorder_rows(w, j):
        for t in range(nt):
            perm_f[j, t] = w[:, t * LANES:(t + 1) * LANES].astype(F32)
        return jnp.concatenate(
            [jnp.concatenate([perm_f[j, t, pl.ds(d, B_HEADS, stride=dB), :] for d in range(dB)], axis=0)
             for t in range(nt)], axis=1).astype(BF16)

    def project_kv(xb, j, scr, lo):
        y = _nn(xb, _unpack(bqkv_p[j]))
        for t in range(nt):
            scr[t, lo:lo + xb.shape[0], :] = y[:, t * LANES:(t + 1) * LANES]

    def project_q(xb, r0, lo):
        n = xb.shape[0]
        q_scr[lo:lo + n, :] = _nn(xb, _unpack(bqkv_p[0])) * b_scale
        g = jax.nn.sigmoid(jnp.sum(xb.astype(F32) * gate, axis=-1, keepdims=True))
        g_scr[pl.ds(r0 + lo, n), :] = jnp.broadcast_to(g, (n, LANES))

    gate = gate_ref[...].astype(F32).reshape(1, D)
    h_scr[0:M, :] = mem0_ref[...].astype(F32)

    bqkv_copy(1).wait()
    bqkv_copy(2).start()
    bqkv_copy(0).start()
    cp_bwo.start()
    bqkv_p[1] = _pack(reorder_rows(bqkv_v[1].T, 1).T)
    bqkv_copy(2).wait()
    x_copy(0).wait()
    w_start(0)
    bqkv_p[2] = _pack(reorder_rows(bqkv_v[2].T, 2).T)
    project_kv(x_v[0:R, :], 1, k_scr, HALO)
    h_scr[M:L, :] = x_v[0:seg, :].astype(F32)
    bqkv_copy(0).wait()
    x_copy(1).start()
    bqkv_p[0] = _pack(reorder_rows(bqkv_v[0].T, 0).T)
    project_kv(x_v[0:R, :], 2, v_scr, HALO)
    cp_bwo.wait()
    bwo_p[...] = _pack(reorder_rows(bwo_v[...], 3))

    for t in range(nt):
        k_scr[t, 0:HALO, :] = jnp.broadcast_to(k_scr[t, HALO:HALO + 1, :], (HALO, LANES))
        v_scr[t, 0:HALO, :] = jnp.broadcast_to(v_scr[t, HALO:HALO + 1, :], (HALO, LANES))

    def stage_pair(c, i):
        for j in range(3):
            wqkv_p[c * ppc + i, :, j * PW:(j + 1) * PW] = _pack(stage[c, j, i * PW:(i + 1) * PW, :].T)

    def a_first(c, kind, i, qkv, pr):
        if kind == "T":
            stage_pair(c, i)
        elif kind == "Q":
            qkv[i] = a_project(c * ppc + i)
        elif kind == "S":
            pr[i] = a_probs(qkv[i][0], qkv[i][1])
        else:
            o_scr[c * ppc + i] = _nn(pr[i], qkv[i][2])

    def b_chunk(c, order):
        r0 = pl.multiple_of(c * R, R)

        def project(i, kv=True):
            xb = x_v[pl.ds(r0 + i * RS, RS), :]
            if kv:
                project_kv(xb, 1, k_scr, HALO + i * RS)
                project_kv(xb, 2, v_scr, HALO + i * RS)
            project_q(xb, r0, i * RS)

        def attend(i):
            for u in range(i * RS, (i + 1) * RS, RA):
                qs = [q_scr[u:u + RA, t * LANES:(t + 1) * LANES] for t in range(nt)]
                logits = []
                for w in range(B_WIN):
                    off = u + HALO - B_DIL * w
                    acc = qs[0] * k_scr[0, off:off + RA, :]
                    for t in range(1, nt):
                        acc = acc + qs[t] * k_scr[t, off:off + RA, :]
                    acc = acc + pltpu.roll(acc, 2 * B_HEADS, 1)
                    acc = acc + pltpu.roll(acc, B_HEADS, 1)
                    if u < B_DIL * w:
                        pos = r0 + u + jax.lax.broadcasted_iota(I32, (RA, LANES), 0)
                        acc = jnp.where(pos >= B_DIL * w, acc, NEG)
                    logits.append(acc)
                mx = functools.reduce(jnp.maximum, logits)
                es = [jnp.exp(l - mx) for l in logits]
                inv = 1.0 / functools.reduce(jnp.add, es)
                for t in range(nt):
                    acc = es[0] * v_scr[t, u + HALO:u + HALO + RA, :]
                    for w in range(1, B_WIN):
                        off = u + HALO - B_DIL * w
                        acc = acc + es[w] * v_scr[t, off:off + RA, :]
                    ob_scr[u // 2:(u + RA) // 2, t * LANES:(t + 1) * LANES] = _pack((acc * inv).astype(BF16))

        def mix(i):
            bb = _nn(_unpack(ob_scr[i * RS // 2:(i + 1) * RS // 2, :]), _unpack(bwo_p[...]))
            rows = pl.ds(r0 + i * RS, RS)
            b_scr[rows, :] = (1.0 - jnp.concatenate([g_scr[rows, :]] * nt, axis=1)) * bb

        qkv, pr = {}, {}
        for op in order.split():
            kind, i = op[0], int(op[1:])
            if kind == "w":
                w_start(i)
            elif kind in "pqam":
                {"p": project, "q": functools.partial(project, kv=False), "a": attend, "m": mix}[kind](i)
            else:
                a_first(c - 1, kind, i, qkv, pr)

    b_chunk(0, B_ORDER_FIRST)

    def b_body(c, carry):
        x_copy(c).wait()
        for j in range(3):
            w_copy(c - 1, j).wait()

        @pl.when(c + 1 < n_chunk)
        def _():
            x_copy(c + 1).start()
            w_start(c + 1)

        for k, when in enumerate(WO_ISSUE):
            pl.when(c == when)(lambda k=k: wo_copy(k).start())

        for t in range(nt):
            k_scr[t, 0:HALO, :] = k_scr[t, R:R + HALO, :]
            v_scr[t, 0:HALO, :] = v_scr[t, R:R + HALO, :]
        b_chunk(c, B_ORDER)
        return carry

    jax.lax.fori_loop(1, n_chunk, b_body, 0)

    n_early = WO_ISSUE.index(n_chunk - 1)
    for j in range(3):
        w_copy(n_chunk - 1, j).wait()
    for c in range(n_early):
        wo_copy(c).wait()

    def repack_wo(p):
        c, i = divmod(p, ppc)
        if (c, i) == (n_early, 0):
            for k in range(n_early, n_chunk):
                wo_copy(k).wait()
        wo_p[p] = _pack(wo_v[c, i * PW:(i + 1) * PW, :])

    qkv0, pr0, acc0 = {}, {}, None
    repack_wo(0)
    for op in LAST_ORDER.split():
        kind, i = op[0], int(op[1:])
        if kind == "O":
            repack_wo(i + 1)
            acc0 = a_out_proj(i, acc0, 0, D)
        else:
            a_first(n_chunk - 1, kind, i, qkv0, pr0)
    repack_wo(n_pair - 1)
    a_finish(0, acc0, n_pair - ppc)
    out_copy(0, seg).start()

    def a_step(s):
        r0 = pl.multiple_of(s * seg, seg)
        h_scr[M:L, :] = x_v[pl.ds(r0, seg), :].astype(F32)

        qkv, pr, acc, n_out = {}, {}, None, 0
        for t in range(n_pair + 2):
            if t < n_pair:
                qkv[t] = a_project(t)
            else:
                for _ in range(3):
                    acc = a_out_proj(n_out, acc, 0, D)
                    n_out += 1
            if 0 <= t - 1 < n_pair:
                pr[t - 1] = a_probs(qkv[t - 1][0], qkv[t - 1][1])
            if 0 <= t - 2 < n_pair:
                o_scr[t - 2] = _nn(pr.pop(t - 2), qkv.pop(t - 2)[2])
        for p in range(n_out, n_pair - A_TAIL):
            acc = a_out_proj(p, acc, 0, D)
        a_finish(r0, acc, n_pair - A_TAIL)

    def a_body(i, carry):
        s0 = 1 + i * A_UNROLL
        for u in range(A_UNROLL):
            a_step(s0 + u)
        out_copy(pl.multiple_of(s0 * seg, seg), A_UNROLL * seg).start()
        return carry

    assert (n_seg - 1) % A_UNROLL == 0
    jax.lax.fori_loop(0, (n_seg - 1) // A_UNROLL, a_body, 0)
    pltpu.make_async_copy(out_v, out_hbm, out_sem).wait()


@functools.partial(jax.jit, static_argnames=("A_seg_len",))
def pallas_gated_mix__memory_aug_recurrent_mem_tr__sliding_local_dilated__prompt_kernel(
    A_x: jax.Array,
    A_mem0: jax.Array,
    A_Wq: jax.Array,
    A_Wk: jax.Array,
    A_Wv: jax.Array,
    A_Wo: jax.Array,
    A_seg_len: int,
    B_x: jax.Array,
    B_wqkv: jax.Array,
    B_wo: jax.Array,
    gate_w: jax.Array,
):
    del B_x
    Bsz, S, D = A_x.shape
    _, H, Dh = A_Wq.shape
    M = A_mem0.shape[1]
    seg = int(A_seg_len)
    assert Bsz == 1 and S % seg == 0 and H % 2 == 0 and (2 * Dh) % LANES == 0 and D % LANES == 0
    n_chunk = 8
    n_pair = H // 2
    PW = 2 * Dh
    R = S // n_chunk
    L = M + seg

    def head_major(w):
        return jnp.transpose(w, (1, 2, 0)).reshape(H * Dh, D)

    any_spec = pl.BlockSpec(memory_space=pl.ANY)
    vmem_spec = pl.BlockSpec(memory_space=pltpu.VMEM)
    out = pl.pallas_call(
        functools.partial(_kernel, S=S, D=D, H=H, Dh=Dh, M=M, seg=seg,
                          n_chunk=n_chunk),
        out_shape=jax.ShapeDtypeStruct((S, D), A_x.dtype),
        in_specs=[any_spec, vmem_spec, any_spec, any_spec, any_spec, any_spec,
                  any_spec, any_spec, vmem_spec],
        out_specs=any_spec,
        scratch_shapes=[
            pltpu.VMEM((S, D), BF16),
            pltpu.VMEM((3, D, D), BF16),
            pltpu.VMEM((D, D), BF16),
            pltpu.VMEM((4, D // LANES, D, LANES), F32),
            pltpu.VMEM((3, D // 2, D), I32),
            pltpu.VMEM((D // 2, D), I32),
            pltpu.VMEM((R, D), F32),
            pltpu.VMEM((D // LANES, HALO + R, LANES), F32),
            pltpu.VMEM((D // LANES, HALO + R, LANES), F32),
            pltpu.VMEM((R // 2, D), I32),
            pltpu.VMEM((S, LANES), F32),
            pltpu.VMEM((S, D), F32),
            pltpu.VMEM((n_chunk, 3, n_pair // n_chunk * PW, D), BF16),
            pltpu.VMEM((n_chunk, n_pair // n_chunk * PW, D), BF16),
            pltpu.VMEM((n_pair, D // 2, 3 * PW), I32),
            pltpu.VMEM((n_pair, PW // 2, D), I32),
            pltpu.VMEM((L, D), F32),
            pltpu.VMEM((n_pair, L, PW), F32),
            pltpu.VMEM((S, D), A_x.dtype),
            pltpu.SemaphoreType.DMA((4,)),
            pltpu.SemaphoreType.DMA((n_chunk,)),
            pltpu.SemaphoreType.DMA((n_chunk, 3)),
            pltpu.SemaphoreType.DMA((n_chunk,)),
            pltpu.SemaphoreType.DMA(()),
        ],
        compiler_params=pltpu.CompilerParams(vmem_limit_bytes=110 * 1024 * 1024),
    )(
        A_x.reshape(S, D),
        A_mem0.reshape(M, D),
        head_major(A_Wq),
        head_major(A_Wk),
        head_major(A_Wv),
        A_Wo.reshape(H * Dh, D),
        B_wqkv,
        B_wo,
        gate_w,
    )
    return out.reshape(Bsz, S, D)
```

```python
import functools

import jax
import jax.numpy as jnp
import jax.experimental.pallas as pl
import jax.experimental.pallas.tpu as pltpu

F32 = jnp.float32
BF16 = jnp.bfloat16
I32 = jnp.int32

LANES = 128
B_HEADS = 32
B_WIN = 8
B_DIL = 2
HALO = 16
NEG = -1000000000.0
RS = 64
RA = 16
A_UNROLL = 3
A_TAIL = 4
B_ORDER = "T0 p0 p1 a0 T1 p2 a1 p3 a2 Q0 Q1 a3 S0 m0 m1 S1 m2 V0 m3 V1"
B_ORDER_FIRST = "q0 q1 a0 q2 a1 q3 w1 a2 m0 a3 m1 m2 m3"
LAST_ORDER = "T0 O0 O1 O2 O3 O4 O5 T1 Q0 O6 O7 S0 Q1 O8 S1 O9 V0 O10 V1 O11 O12 O13"
WO_ISSUE = (1, 2, 3, 4, 5, 6, 7, 7)


def _nt(a, b):
    return jax.lax.dot_general(a, b, (((1,), (1,)), ((), ())), preferred_element_type=F32)


def _nn(a, b):
    return jax.lax.dot_general(a, b, (((1,), (0,)), ((), ())), preferred_element_type=F32)


def _pack(w):
    return pltpu.bitcast(w, I32)


def _unpack(w):
    return pltpu.bitcast(w, BF16)


def _kernel(x_hbm, mem0_ref, wq_hbm, wk_hbm, wv_hbm, wo_hbm, bqkv_hbm, bwo_hbm, gate_ref,
            out_hbm,
            x_v, bqkv_v, bwo_v, perm_f, bqkv_p, bwo_p, q_scr, k_scr, v_scr, ob_scr, g_scr, b_scr,
            stage, wo_v, wqkv_p, wo_p, h_scr, o_scr, out_v,
            in_sem, x_sem, w_sem, wo_sem, out_sem,
            *, S, D, H, Dh, M, seg, n_chunk):
    L = M + seg
    n_seg = S // seg
    n_iter = (n_seg - 1) // A_UNROLL
    n_pair = H // 2
    PW = 2 * Dh
    R = S // n_chunk
    ppc = n_pair // n_chunk
    nt = D // LANES
    dB = D // B_HEADS
    a_scale = Dh ** (-0.5)
    b_scale = dB ** (-0.5)

    def bqkv_copy(j):
        cols = pl.ds(j * D, D)
        return pltpu.make_async_copy(bqkv_hbm.at[:, cols], bqkv_v.at[j], in_sem.at[j])

    cp_bwo = pltpu.make_async_copy(bwo_hbm, bwo_v, in_sem.at[3])

    def x_copy(c):
        rows = pl.ds(pl.multiple_of(c * R, R), R)
        return pltpu.make_async_copy(x_hbm.at[rows, :], x_v.at[rows, :], x_sem.at[c])

    def chunk_rows(c):
        return pl.ds(pl.multiple_of(c * (ppc * PW), ppc * PW), ppc * PW)

    def w_copy(c, j):
        src = (wq_hbm, wk_hbm, wv_hbm)[j]
        return pltpu.make_async_copy(src.at[chunk_rows(c), :], stage.at[c, j], w_sem.at[c, j])

    def wo_copy(c):
        return pltpu.make_async_copy(wo_hbm.at[chunk_rows(c), :], wo_v.at[c], wo_sem.at[c])

    def w_start(c):
        for j in range(3):
            w_copy(c, j).start()

    def out_copy(slot, row0, n):
        rows = pl.ds(row0, n)
        return pltpu.make_async_copy(out_v.at[rows, :], out_hbm.at[rows, :], out_sem.at[slot])

    def block_diag(z):
        in_a = jax.lax.broadcasted_iota(I32, (L, PW), 1) < Dh
        return jnp.concatenate([jnp.where(in_a, z, 0.0), jnp.where(in_a, 0.0, z)], axis=0).astype(BF16)

    def a_project(p):
        qkv = _nn(h_scr[...], _unpack(wqkv_p[p]))
        return qkv[:, 0:PW], block_diag(qkv[:, PW:2 * PW]), block_diag(qkv[:, 2 * PW:3 * PW])

    def a_probs(q, kbd):
        row = jax.lax.broadcasted_iota(I32, (L, 2 * L), 0)
        col = jax.lax.broadcasted_iota(I32, (L, 2 * L), 1)
        first = col < L
        visible = (row < M) | (row >= jnp.where(first, col, col - L))
        sc = jnp.where(visible, _nt(q, kbd) * a_scale, NEG)
        m_a = jnp.max(jnp.where(first, sc, -jnp.inf), axis=-1, keepdims=True)
        m_b = jnp.max(jnp.where(first, -jnp.inf, sc), axis=-1, keepdims=True)
        e = jnp.exp(sc - jnp.where(first, m_a, m_b))
        l_a = jnp.sum(jnp.where(first, e, 0.0), axis=-1, keepdims=True)
        l_b = jnp.sum(jnp.where(first, 0.0, e), axis=-1, keepdims=True)
        return e * jnp.where(first, 1.0 / l_a, 1.0 / l_b)

    def a_out_proj(p, acc, lo, hi):
        y = _nn(o_scr[p], _unpack(wo_p[p, :, lo:hi]))
        return y if acc is None else acc + y

    def a_finish(r0, acc, p0):
        g = g_scr[pl.ds(r0, seg), :]
        for lo, hi in ((0, D - LANES), (D - LANES, D)):
            part = acc[:, lo:hi]
            for p in range(p0, n_pair):
                part = a_out_proj(p, part, lo, hi)
            h_scr[0:M, lo:hi] = part[0:M, :]
            gg = jnp.concatenate([g] * ((hi - lo) // LANES), axis=1)
            out_v[pl.ds(r0, seg), lo:hi] = (gg * part[M:L, :] + b_scr[pl.ds(r0, seg), lo:hi]).astype(out_v.dtype)

    bqkv_copy(1).start()
    x_copy(0).start()

    def reorder_rows(w, j):
        for t in range(nt):
            perm_f[j, t] = w[:, t * LANES:(t + 1) * LANES].astype(F32)
        return jnp.concatenate(
            [jnp.concatenate([perm_f[j, t, pl.ds(d, B_HEADS, stride=dB), :] for d in range(dB)], axis=0)
             for t in range(nt)], axis=1).astype(BF16)

    def project_kv(xb, j, scr, lo):
        y = _nn(xb, _unpack(bqkv_p[j]))
        for t in range(nt):
            scr[t, lo:lo + xb.shape[0], :] = y[:, t * LANES:(t + 1) * LANES]

    def project_q(xb, r0, lo):
        n = xb.shape[0]
        q_scr[lo:lo + n, :] = _nn(xb, _unpack(bqkv_p[0])) * b_scale
        g = jax.nn.sigmoid(jnp.sum(xb.astype(F32) * gate, axis=-1, keepdims=True))
        g_scr[pl.ds(r0 + lo, n), :] = jnp.broadcast_to(g, (n, LANES))

    gate = gate_ref[...].astype(F32).reshape(1, D)
    h_scr[0:M, :] = mem0_ref[...].astype(F32)

    bqkv_copy(1).wait()
    bqkv_copy(2).start()
    bqkv_copy(0).start()
    cp_bwo.start()
    bqkv_p[1] = _pack(reorder_rows(bqkv_v[1].T, 1).T)
    bqkv_copy(2).wait()
    x_copy(0).wait()
    w_start(0)
    bqkv_p[2] = _pack(reorder_rows(bqkv_v[2].T, 2).T)
    project_kv(x_v[0:R, :], 1, k_scr, HALO)
    h_scr[M:L, :] = x_v[0:seg, :].astype(F32)
    bqkv_copy(0).wait()
    x_copy(1).start()
    bqkv_p[0] = _pack(reorder_rows(bqkv_v[0].T, 0).T)
    project_kv(x_v[0:R, :], 2, v_scr, HALO)
    cp_bwo.wait()
    bwo_p[...] = _pack(reorder_rows(bwo_v[...], 3))

    for t in range(nt):
        k_scr[t, 0:HALO, :] = jnp.broadcast_to(k_scr[t, HALO:HALO + 1, :], (HALO, LANES))
        v_scr[t, 0:HALO, :] = jnp.broadcast_to(v_scr[t, HALO:HALO + 1, :], (HALO, LANES))

    def stage_pair(c, i):
        for j in range(3):
            wqkv_p[c * ppc + i, :, j * PW:(j + 1) * PW] = _pack(stage[c, j, i * PW:(i + 1) * PW, :].T)

    def a_first(c, kind, i, qkv, pr):
        if kind == "T":
            stage_pair(c, i)
        elif kind == "Q":
            qkv[i] = a_project(c * ppc + i)
        elif kind == "S":
            pr[i] = a_probs(qkv[i][0], qkv[i][1])
        else:
            o_scr[c * ppc + i] = _nn(pr[i], qkv[i][2])

    def b_chunk(c, order):
        r0 = pl.multiple_of(c * R, R)

        def project(i, kv=True):
            xb = x_v[pl.ds(r0 + i * RS, RS), :]
            if kv:
                project_kv(xb, 1, k_scr, HALO + i * RS)
                project_kv(xb, 2, v_scr, HALO + i * RS)
            project_q(xb, r0, i * RS)

        def attend(i):
            for u in range(i * RS, (i + 1) * RS, RA):
                qs = [q_scr[u:u + RA, t * LANES:(t + 1) * LANES] for t in range(nt)]
                logits = []
                for w in range(B_WIN):
                    off = u + HALO - B_DIL * w
                    acc = qs[0] * k_scr[0, off:off + RA, :]
                    for t in range(1, nt):
                        acc = acc + qs[t] * k_scr[t, off:off + RA, :]
                    acc = acc + pltpu.roll(acc, 2 * B_HEADS, 1)
                    acc = acc + pltpu.roll(acc, B_HEADS, 1)
                    if u < B_DIL * w:
                        pos = r0 + u + jax.lax.broadcasted_iota(I32, (RA, LANES), 0)
                        acc = jnp.where(pos >= B_DIL * w, acc, NEG)
                    logits.append(acc)
                mx = functools.reduce(jnp.maximum, logits)
                es = [jnp.exp(l - mx) for l in logits]
                inv = 1.0 / functools.reduce(jnp.add, es)
                for t in range(nt):
                    acc = es[0] * v_scr[t, u + HALO:u + HALO + RA, :]
                    for w in range(1, B_WIN):
                        off = u + HALO - B_DIL * w
                        acc = acc + es[w] * v_scr[t, off:off + RA, :]
                    ob_scr[u // 2:(u + RA) // 2, t * LANES:(t + 1) * LANES] = _pack((acc * inv).astype(BF16))

        def mix(i):
            bb = _nn(_unpack(ob_scr[i * RS // 2:(i + 1) * RS // 2, :]), _unpack(bwo_p[...]))
            rows = pl.ds(r0 + i * RS, RS)
            b_scr[rows, :] = (1.0 - jnp.concatenate([g_scr[rows, :]] * nt, axis=1)) * bb

        qkv, pr = {}, {}
        for op in order.split():
            kind, i = op[0], int(op[1:])
            if kind == "w":
                w_start(i)
            elif kind in "pqam":
                {"p": project, "q": functools.partial(project, kv=False), "a": attend, "m": mix}[kind](i)
            else:
                a_first(c - 1, kind, i, qkv, pr)

    b_chunk(0, B_ORDER_FIRST)

    def b_body(c, carry):
        x_copy(c).wait()
        for j in range(3):
            w_copy(c - 1, j).wait()

        @pl.when(c + 1 < n_chunk)
        def _():
            x_copy(c + 1).start()
            w_start(c + 1)

        for k, when in enumerate(WO_ISSUE):
            pl.when(c == when)(lambda k=k: wo_copy(k).start())

        for t in range(nt):
            k_scr[t, 0:HALO, :] = k_scr[t, R:R + HALO, :]
            v_scr[t, 0:HALO, :] = v_scr[t, R:R + HALO, :]
        b_chunk(c, B_ORDER)
        return carry

    jax.lax.fori_loop(1, n_chunk, b_body, 0)

    n_early = WO_ISSUE.index(n_chunk - 1)
    for j in range(3):
        w_copy(n_chunk - 1, j).wait()
    for c in range(n_early):
        wo_copy(c).wait()

    def repack_wo(p):
        c, i = divmod(p, ppc)
        if (c, i) == (n_early, 0):
            for k in range(n_early, n_chunk):
                wo_copy(k).wait()
        wo_p[p] = _pack(wo_v[c, i * PW:(i + 1) * PW, :])

    qkv0, pr0, acc0 = {}, {}, None
    repack_wo(0)
    for op in LAST_ORDER.split():
        kind, i = op[0], int(op[1:])
        if kind == "O":
            repack_wo(i + 1)
            acc0 = a_out_proj(i, acc0, 0, D)
        else:
            a_first(n_chunk - 1, kind, i, qkv0, pr0)
    repack_wo(n_pair - 1)
    a_finish(0, acc0, n_pair - ppc)
    out_copy(n_iter, 0, seg).start()

    def a_step(s):
        r0 = pl.multiple_of(s * seg, seg)
        h_scr[M:L, :] = x_v[pl.ds(r0, seg), :].astype(F32)

        qkv, pr, acc, n_out = {}, {}, None, 0
        for t in range(n_pair + 2):
            if t < n_pair:
                qkv[t] = a_project(t)
            else:
                for _ in range(3):
                    acc = a_out_proj(n_out, acc, 0, D)
                    n_out += 1
            if 0 <= t - 1 < n_pair:
                pr[t - 1] = a_probs(qkv[t - 1][0], qkv[t - 1][1])
            if 0 <= t - 2 < n_pair:
                o_scr[t - 2] = _nn(pr.pop(t - 2), qkv.pop(t - 2)[2])
        for p in range(n_out, n_pair - A_TAIL):
            acc = a_out_proj(p, acc, 0, D)
        a_finish(r0, acc, n_pair - A_TAIL)

    def a_body(i, carry):
        s0 = 1 + i * A_UNROLL
        for u in range(A_UNROLL):
            a_step(s0 + u)
        out_copy(i, pl.multiple_of(s0 * seg, seg), A_UNROLL * seg).start()
        return carry

    jax.lax.fori_loop(0, n_iter, a_body, 0)
    out_copy(n_iter, 0, seg).wait()
    for i in range(n_iter):
        out_copy(i, (1 + i * A_UNROLL) * seg, A_UNROLL * seg).wait()


@functools.partial(jax.jit, static_argnames=("A_seg_len",))
def pallas_gated_mix__memory_aug_recurrent_mem_tr__sliding_local_dilated__prompt_kernel(
    A_x: jax.Array,
    A_mem0: jax.Array,
    A_Wq: jax.Array,
    A_Wk: jax.Array,
    A_Wv: jax.Array,
    A_Wo: jax.Array,
    A_seg_len: int,
    B_x: jax.Array,
    B_wqkv: jax.Array,
    B_wo: jax.Array,
    gate_w: jax.Array,
):
    del B_x
    Bsz, S, D = A_x.shape
    _, H, Dh = A_Wq.shape
    M = A_mem0.shape[1]
    seg = int(A_seg_len)
    assert Bsz == 1 and S % seg == 0 and H % 2 == 0 and (2 * Dh) % LANES == 0 and D % LANES == 0
    n_chunk = len(WO_ISSUE)
    n_pair = H // 2
    PW = 2 * Dh
    R = S // n_chunk
    L = M + seg
    assert (S // seg - 1) % A_UNROLL == 0 and R == 4 * RS and n_pair == 2 * n_chunk
    assert 4 * B_HEADS == LANES and L % 8 == 0 and 2 * L <= LANES

    def head_major(w):
        return jnp.transpose(w, (1, 2, 0)).reshape(H * Dh, D)

    any_spec = pl.BlockSpec(memory_space=pl.ANY)
    vmem_spec = pl.BlockSpec(memory_space=pltpu.VMEM)
    out = pl.pallas_call(
        functools.partial(_kernel, S=S, D=D, H=H, Dh=Dh, M=M, seg=seg,
                          n_chunk=n_chunk),
        out_shape=jax.ShapeDtypeStruct((S, D), A_x.dtype),
        in_specs=[any_spec, vmem_spec, any_spec, any_spec, any_spec, any_spec,
                  any_spec, any_spec, vmem_spec],
        out_specs=any_spec,
        scratch_shapes=[
            pltpu.VMEM((S, D), BF16),
            pltpu.VMEM((3, D, D), BF16),
            pltpu.VMEM((D, D), BF16),
            pltpu.VMEM((4, D // LANES, D, LANES), F32),
            pltpu.VMEM((3, D // 2, D), I32),
            pltpu.VMEM((D // 2, D), I32),
            pltpu.VMEM((R, D), F32),
            pltpu.VMEM((D // LANES, HALO + R, LANES), F32),
            pltpu.VMEM((D // LANES, HALO + R, LANES), F32),
            pltpu.VMEM((R // 2, D), I32),
            pltpu.VMEM((S, LANES), F32),
            pltpu.VMEM((S, D), F32),
            pltpu.VMEM((n_chunk, 3, n_pair // n_chunk * PW, D), BF16),
            pltpu.VMEM((n_chunk, n_pair // n_chunk * PW, D), BF16),
            pltpu.VMEM((n_pair, D // 2, 3 * PW), I32),
            pltpu.VMEM((n_pair, PW // 2, D), I32),
            pltpu.VMEM((L, D), F32),
            pltpu.VMEM((n_pair, L, PW), F32),
            pltpu.VMEM((S, D), A_x.dtype),
            pltpu.SemaphoreType.DMA((4,)),
            pltpu.SemaphoreType.DMA((n_chunk,)),
            pltpu.SemaphoreType.DMA((n_chunk, 3)),
            pltpu.SemaphoreType.DMA((n_chunk,)),
            pltpu.SemaphoreType.DMA(((S // seg - 1) // A_UNROLL + 1,)),
        ],
        compiler_params=pltpu.CompilerParams(vmem_limit_bytes=110 * 1024 * 1024),
    )(
        A_x.reshape(S, D),
        A_mem0.reshape(M, D),
        head_major(A_Wq),
        head_major(A_Wk),
        head_major(A_Wv),
        A_Wo.reshape(H * Dh, D),
        B_wqkv,
        B_wo,
        gate_w,
    )
    return out.reshape(Bsz, S, D)
```

```python
import functools

import jax
import jax.numpy as jnp
import jax.experimental.pallas as pl
import jax.experimental.pallas.tpu as pltpu

F32 = jnp.float32
BF16 = jnp.bfloat16
I32 = jnp.int32

LANES = 128
B_HEADS = 32
B_WIN = 8
B_DIL = 2
HALO = 16
NEG = -1000000000.0
RS = 64
RA = 16
A_UNROLL = 3
A_TAIL = 4
B_ORDER = "T0 p0 p1 a0 T1 p2 a1 p3 a2 Q0 Q1 a3 S0 m0 m1 S1 m2 V0 m3 V1"
B_ORDER_FIRST = "q0 q1 a0 q2 a1 q3 w1 a2 m0 a3 m1 m2 m3"
LAST_ORDER = "T0 O0 O1 O2 O3 O4 O5 T1 Q0 O6 O7 S0 Q1 O8 S1 O9 V0 O10 V1 O11 O12 O13"
WO_ISSUE = (1, 2, 3, 4, 5, 6, 7, 7)


def _nt(a, b):
    return jax.lax.dot_general(a, b, (((1,), (1,)), ((), ())), preferred_element_type=F32)


def _nn(a, b):
    return jax.lax.dot_general(a, b, (((1,), (0,)), ((), ())), preferred_element_type=F32)


def _pack(w):
    return pltpu.bitcast(w, I32)


def _unpack(w):
    return pltpu.bitcast(w, BF16)


def _kernel(x_hbm, mem0_ref, wq_hbm, wk_hbm, wv_hbm, wo_hbm, bqkv_hbm, bwo_hbm, gate_ref,
            out_hbm,
            x_v, bqkv_v, bwo_v, perm_f, bqkv_p, bwo_p, q_scr, k_scr, v_scr, ob_scr, g_scr, b_scr,
            stage, wo_v, wqkv_p, wo_p, h_scr, o_scr, out_v,
            in_sem, x_sem, w_sem, wo_sem, out_sem,
            *, S, D, H, Dh, M, seg, n_chunk):
    L = M + seg
    n_seg = S // seg
    n_iter = (n_seg - 1) // A_UNROLL
    n_pair = H // 2
    PW = 2 * Dh
    R = S // n_chunk
    ppc = n_pair // n_chunk
    nt = D // LANES
    dB = D // B_HEADS
    a_scale = Dh ** (-0.5)
    b_scale = dB ** (-0.5)

    def bqkv_copy(j):
        cols = pl.ds(j * D, D)
        return pltpu.make_async_copy(bqkv_hbm.at[:, cols], bqkv_v.at[j], in_sem.at[j])

    cp_bwo = pltpu.make_async_copy(bwo_hbm, bwo_v, in_sem.at[3])

    def x_copy(c):
        rows = pl.ds(pl.multiple_of(c * R, R), R)
        return pltpu.make_async_copy(x_hbm.at[rows, :], x_v.at[rows, :], x_sem.at[c])

    def chunk_rows(c):
        return pl.ds(pl.multiple_of(c * (ppc * PW), ppc * PW), ppc * PW)

    def w_copy(c, j):
        src = (wq_hbm, wk_hbm, wv_hbm)[j]
        return pltpu.make_async_copy(src.at[chunk_rows(c), :], stage.at[c, j], w_sem.at[c, j])

    def wo_copy(c):
        return pltpu.make_async_copy(wo_hbm.at[chunk_rows(c), :], wo_v.at[c], wo_sem.at[c])

    def w_start(c):
        for j in range(3):
            w_copy(c, j).start()

    def out_copy(slot, row0, n):
        rows = pl.ds(row0, n)
        return pltpu.make_async_copy(out_v.at[rows, :], out_hbm.at[rows, :], out_sem.at[slot])

    def block_diag(z):
        in_a = jax.lax.broadcasted_iota(I32, (L, PW), 1) < Dh
        return jnp.concatenate([jnp.where(in_a, z, 0.0), jnp.where(in_a, 0.0, z)], axis=0).astype(BF16)

    def a_project(p):
        qkv = _nn(h_scr[...], _unpack(wqkv_p[p]))
        return qkv[:, 0:PW], block_diag(qkv[:, PW:2 * PW]), block_diag(qkv[:, 2 * PW:3 * PW])

    def a_probs(q, kbd):
        row = jax.lax.broadcasted_iota(I32, (L, 2 * L), 0)
        col = jax.lax.broadcasted_iota(I32, (L, 2 * L), 1)
        first = col < L
        visible = (row < M) | (row >= jnp.where(first, col, col - L))
        sc = jnp.where(visible, _nt(q, kbd) * a_scale, NEG)
        m_a = jnp.max(jnp.where(first, sc, -jnp.inf), axis=-1, keepdims=True)
        m_b = jnp.max(jnp.where(first, -jnp.inf, sc), axis=-1, keepdims=True)
        e = jnp.exp(sc - jnp.where(first, m_a, m_b))
        l_a = jnp.sum(jnp.where(first, e, 0.0), axis=-1, keepdims=True)
        l_b = jnp.sum(jnp.where(first, 0.0, e), axis=-1, keepdims=True)
        return e * jnp.where(first, 1.0 / l_a, 1.0 / l_b)

    def a_out_proj(p, acc, lo, hi):
        y = _nn(o_scr[p], _unpack(wo_p[p, :, lo:hi]))
        return y if acc is None else acc + y

    def a_finish(r0, acc, p0):
        g = g_scr[pl.ds(r0, seg), :]
        for lo, hi in ((0, D - LANES), (D - LANES, D)):
            part = acc[:, lo:hi]
            for p in range(p0, n_pair):
                part = a_out_proj(p, part, lo, hi)
            h_scr[0:M, lo:hi] = part[0:M, :]
            gg = jnp.concatenate([g] * ((hi - lo) // LANES), axis=1)
            out_v[pl.ds(r0, seg), lo:hi] = (gg * part[M:L, :] + b_scr[pl.ds(r0, seg), lo:hi]).astype(out_v.dtype)

    bqkv_copy(1).start()
    x_copy(0).start()

    def reorder_rows(w, j):
        for t in range(nt):
            perm_f[j, t] = w[:, t * LANES:(t + 1) * LANES].astype(F32)
        return jnp.concatenate(
            [jnp.concatenate([perm_f[j, t, pl.ds(d, B_HEADS, stride=dB), :] for d in range(dB)], axis=0)
             for t in range(nt)], axis=1).astype(BF16)

    def project_kv(xb, j, scr, lo):
        y = _nn(xb, _unpack(bqkv_p[j]))
        for t in range(nt):
            scr[t, lo:lo + xb.shape[0], :] = y[:, t * LANES:(t + 1) * LANES]

    def project_q(xb, r0, lo):
        n = xb.shape[0]
        q_scr[lo:lo + n, :] = _nn(xb, _unpack(bqkv_p[0])) * b_scale
        g = jax.nn.sigmoid(jnp.sum(xb.astype(F32) * gate, axis=-1, keepdims=True))
        g_scr[pl.ds(r0 + lo, n), :] = jnp.broadcast_to(g, (n, LANES))

    gate = gate_ref[...].astype(F32).reshape(1, D)
    h_scr[0:M, :] = mem0_ref[...].astype(F32)

    bqkv_copy(1).wait()
    bqkv_copy(2).start()
    bqkv_copy(0).start()
    cp_bwo.start()
    bqkv_p[1] = _pack(reorder_rows(bqkv_v[1].T, 1).T)
    bqkv_copy(2).wait()
    x_copy(0).wait()
    w_start(0)
    bqkv_p[2] = _pack(reorder_rows(bqkv_v[2].T, 2).T)
    project_kv(x_v[0:R, :], 1, k_scr, HALO)
    h_scr[M:L, :] = x_v[0:seg, :].astype(F32)
    bqkv_copy(0).wait()
    x_copy(1).start()
    bqkv_p[0] = _pack(reorder_rows(bqkv_v[0].T, 0).T)
    project_kv(x_v[0:R, :], 2, v_scr, HALO)
    cp_bwo.wait()
    bwo_p[...] = _pack(reorder_rows(bwo_v[...], 3))

    for t in range(nt):
        k_scr[t, 0:HALO, :] = jnp.broadcast_to(k_scr[t, HALO:HALO + 1, :], (HALO, LANES))
        v_scr[t, 0:HALO, :] = jnp.broadcast_to(v_scr[t, HALO:HALO + 1, :], (HALO, LANES))

    def stage_pair(c, i):
        for j in range(3):
            wqkv_p[c * ppc + i, :, j * PW:(j + 1) * PW] = _pack(stage[c, j, i * PW:(i + 1) * PW, :].T)

    def a_first(c, kind, i, qkv, pr):
        if kind == "T":
            stage_pair(c, i)
        elif kind == "Q":
            qkv[i] = a_project(c * ppc + i)
        elif kind == "S":
            pr[i] = a_probs(qkv[i][0], qkv[i][1])
        else:
            o_scr[c * ppc + i] = _nn(pr[i], qkv[i][2])

    def b_chunk(c, order):
        r0 = pl.multiple_of(c * R, R)

        def project(i, kv=True):
            xb = x_v[pl.ds(r0 + i * RS, RS), :]
            if kv:
                project_kv(xb, 1, k_scr, HALO + i * RS)
                project_kv(xb, 2, v_scr, HALO + i * RS)
            project_q(xb, r0, i * RS)

        def attend(i):
            for u in range(i * RS, (i + 1) * RS, RA):
                qs = [q_scr[u:u + RA, t * LANES:(t + 1) * LANES] for t in range(nt)]
                logits = []
                for w in range(B_WIN):
                    off = u + HALO - B_DIL * w
                    acc = qs[0] * k_scr[0, off:off + RA, :]
                    for t in range(1, nt):
                        acc = acc + qs[t] * k_scr[t, off:off + RA, :]
                    acc = acc + pltpu.roll(acc, 2 * B_HEADS, 1)
                    acc = acc + pltpu.roll(acc, B_HEADS, 1)
                    if u < B_DIL * w:
                        pos = r0 + u + jax.lax.broadcasted_iota(I32, (RA, LANES), 0)
                        acc = jnp.where(pos >= B_DIL * w, acc, NEG)
                    logits.append(acc)
                mx = functools.reduce(jnp.maximum, logits)
                es = [jnp.exp(l - mx) for l in logits]
                inv = 1.0 / functools.reduce(jnp.add, es)
                for t in range(nt):
                    acc = es[0] * v_scr[t, u + HALO:u + HALO + RA, :]
                    for w in range(1, B_WIN):
                        off = u + HALO - B_DIL * w
                        acc = acc + es[w] * v_scr[t, off:off + RA, :]
                    ob_scr[u // 2:(u + RA) // 2, t * LANES:(t + 1) * LANES] = _pack((acc * inv).astype(BF16))

        def mix(i):
            bb = _nn(_unpack(ob_scr[i * RS // 2:(i + 1) * RS // 2, :]), _unpack(bwo_p[...]))
            rows = pl.ds(r0 + i * RS, RS)
            b_scr[rows, :] = (1.0 - jnp.concatenate([g_scr[rows, :]] * nt, axis=1)) * bb

        qkv, pr = {}, {}
        for op in order.split():
            kind, i = op[0], int(op[1:])
            if kind == "w":
                w_start(i)
            elif kind in "pqam":
                {"p": project, "q": functools.partial(project, kv=False), "a": attend, "m": mix}[kind](i)
            else:
                a_first(c - 1, kind, i, qkv, pr)

    b_chunk(0, B_ORDER_FIRST)

    def b_body(c, carry):
        x_copy(c).wait()
        for j in range(3):
            w_copy(c - 1, j).wait()

        @pl.when(c + 1 < n_chunk)
        def _():
            x_copy(c + 1).start()
            w_start(c + 1)

        for k, when in enumerate(WO_ISSUE):
            pl.when(c == when)(lambda k=k: wo_copy(k).start())

        for t in range(nt):
            k_scr[t, 0:HALO, :] = k_scr[t, R:R + HALO, :]
            v_scr[t, 0:HALO, :] = v_scr[t, R:R + HALO, :]
        b_chunk(c, B_ORDER)
        return carry

    jax.lax.fori_loop(1, n_chunk, b_body, 0)

    n_early = WO_ISSUE.index(n_chunk - 1)
    for j in range(3):
        w_copy(n_chunk - 1, j).wait()
    for c in range(n_early):
        wo_copy(c).wait()

    def repack_wo(p):
        c, i = divmod(p, ppc)
        if (c, i) == (n_early, 0):
            for k in range(n_early, n_chunk):
                wo_copy(k).wait()
        wo_p[p] = _pack(wo_v[c, i * PW:(i + 1) * PW, :])

    qkv0, pr0, acc0 = {}, {}, None
    repack_wo(0)
    for op in LAST_ORDER.split():
        kind, i = op[0], int(op[1:])
        if kind == "O":
            repack_wo(i + 1)
            acc0 = a_out_proj(i, acc0, 0, D)
        else:
            a_first(n_chunk - 1, kind, i, qkv0, pr0)
    repack_wo(n_pair - 1)
    a_finish(0, acc0, n_pair - ppc)
    out_copy(1, 0, seg).start()

    def a_step(s):
        r0 = pl.multiple_of(s * seg, seg)
        h_scr[M:L, :] = x_v[pl.ds(r0, seg), :].astype(F32)

        qkv, pr, acc, n_out = {}, {}, None, 0
        for t in range(n_pair + 2):
            if t < n_pair:
                qkv[t] = a_project(t)
            else:
                for _ in range(3):
                    acc = a_out_proj(n_out, acc, 0, D)
                    n_out += 1
            if 0 <= t - 1 < n_pair:
                pr[t - 1] = a_probs(qkv[t - 1][0], qkv[t - 1][1])
            if 0 <= t - 2 < n_pair:
                o_scr[t - 2] = _nn(pr.pop(t - 2), qkv.pop(t - 2)[2])
        for p in range(n_out, n_pair - A_TAIL):
            acc = a_out_proj(p, acc, 0, D)
        a_finish(r0, acc, n_pair - A_TAIL)

    def body_copy(i):
        return out_copy(0, pl.multiple_of((1 + i * A_UNROLL) * seg, seg), A_UNROLL * seg)

    def a_body(i, carry):
        s0 = 1 + i * A_UNROLL
        for u in range(A_UNROLL):
            a_step(s0 + u)
        pl.when(i > 0)(lambda: body_copy(i - 1).wait())
        body_copy(i).start()
        return carry

    jax.lax.fori_loop(0, n_iter, a_body, 0)
    out_copy(1, 0, seg).wait()
    body_copy(n_iter - 1).wait()


@functools.partial(jax.jit, static_argnames=("A_seg_len",))
def pallas_gated_mix__memory_aug_recurrent_mem_tr__sliding_local_dilated__prompt_kernel(
    A_x: jax.Array,
    A_mem0: jax.Array,
    A_Wq: jax.Array,
    A_Wk: jax.Array,
    A_Wv: jax.Array,
    A_Wo: jax.Array,
    A_seg_len: int,
    B_x: jax.Array,
    B_wqkv: jax.Array,
    B_wo: jax.Array,
    gate_w: jax.Array,
):
    del B_x
    Bsz, S, D = A_x.shape
    _, H, Dh = A_Wq.shape
    M = A_mem0.shape[1]
    seg = int(A_seg_len)
    assert Bsz == 1 and S % seg == 0 and H % 2 == 0 and (2 * Dh) % LANES == 0 and D % LANES == 0
    n_chunk = len(WO_ISSUE)
    n_pair = H // 2
    PW = 2 * Dh
    R = S // n_chunk
    L = M + seg
    assert (S // seg - 1) % A_UNROLL == 0 and R == 4 * RS and n_pair == 2 * n_chunk
    assert 4 * B_HEADS == LANES and L % 8 == 0 and 2 * L <= LANES

    def head_major(w):
        return jnp.transpose(w, (1, 2, 0)).reshape(H * Dh, D)

    any_spec = pl.BlockSpec(memory_space=pl.ANY)
    vmem_spec = pl.BlockSpec(memory_space=pltpu.VMEM)
    out = pl.pallas_call(
        functools.partial(_kernel, S=S, D=D, H=H, Dh=Dh, M=M, seg=seg,
                          n_chunk=n_chunk),
        out_shape=jax.ShapeDtypeStruct((S, D), A_x.dtype),
        in_specs=[any_spec, vmem_spec, any_spec, any_spec, any_spec, any_spec,
                  any_spec, any_spec, vmem_spec],
        out_specs=any_spec,
        scratch_shapes=[
            pltpu.VMEM((S, D), BF16),
            pltpu.VMEM((3, D, D), BF16),
            pltpu.VMEM((D, D), BF16),
            pltpu.VMEM((4, D // LANES, D, LANES), F32),
            pltpu.VMEM((3, D // 2, D), I32),
            pltpu.VMEM((D // 2, D), I32),
            pltpu.VMEM((R, D), F32),
            pltpu.VMEM((D // LANES, HALO + R, LANES), F32),
            pltpu.VMEM((D // LANES, HALO + R, LANES), F32),
            pltpu.VMEM((R // 2, D), I32),
            pltpu.VMEM((S, LANES), F32),
            pltpu.VMEM((S, D), F32),
            pltpu.VMEM((n_chunk, 3, n_pair // n_chunk * PW, D), BF16),
            pltpu.VMEM((n_chunk, n_pair // n_chunk * PW, D), BF16),
            pltpu.VMEM((n_pair, D // 2, 3 * PW), I32),
            pltpu.VMEM((n_pair, PW // 2, D), I32),
            pltpu.VMEM((L, D), F32),
            pltpu.VMEM((n_pair, L, PW), F32),
            pltpu.VMEM((S, D), A_x.dtype),
            pltpu.SemaphoreType.DMA((4,)),
            pltpu.SemaphoreType.DMA((n_chunk,)),
            pltpu.SemaphoreType.DMA((n_chunk, 3)),
            pltpu.SemaphoreType.DMA((n_chunk,)),
            pltpu.SemaphoreType.DMA((2,)),
        ],
        compiler_params=pltpu.CompilerParams(vmem_limit_bytes=110 * 1024 * 1024),
    )(
        A_x.reshape(S, D),
        A_mem0.reshape(M, D),
        head_major(A_Wq),
        head_major(A_Wk),
        head_major(A_Wv),
        A_Wo.reshape(H * Dh, D),
        B_wqkv,
        B_wo,
        gate_w,
    )
    return out.reshape(Bsz, S, D)
```
